```python
import os as _os
_os.environ.setdefault("JAX_PLATFORMS", "cpu")
import jax
import jax.numpy as jnp

def _softmax(x, axis=-1):
    return jax.nn.softmax(x, axis=axis)
def _gelu(x):
    return jax.nn.gelu(x, approximate=True)
def _silu(x):
    return jax.nn.silu(x)
def _sigmoid(x):
    return jax.nn.sigmoid(x)
def _layernorm(x, axis=-1, eps=1e-5):
    m = jnp.mean(x, axis=axis, keepdims=True)
    v = jnp.var(x, axis=axis, keepdims=True)
    return (x - m) / jnp.sqrt(v + eps)
def _scatter_add(tgt, idx, src, axis=0):
    return tgt.at[idx].add(src)
def _segment_sum(src, seg, n):
    return jax.ops.segment_sum(src, seg, n)
class _Rng:
    def __init__(self, key):
        self._k = key
    def _next(self):
        self._k, sub = jax.random.split(self._k)
        return sub
    def normal(self, shape):
        return jax.random.normal(self._next(), shape, dtype=jnp.bfloat16)
    def randint(self, lo, hi, shape):
        return jax.random.randint(self._next(), shape, lo, hi, dtype=jnp.int32)
    def uniform(self, shape, lo=0.0, hi=1.0):
        return jax.random.uniform(self._next(), shape, jnp.bfloat16, lo, hi)
    def permutation(self, n):
        return jax.random.permutation(self._next(), n)


kernel_name = 'concat_heads__gqa_block_cached__gqa_block_cached__near_ridge'

def setup_inputs():
    _rng = _Rng(jax.random.key(int.from_bytes(__import__("os").urandom(4), "little")))
    _w = (lambda a: (lambda t: t.astype(jnp.bfloat16) if jnp.issubdtype(t.dtype, jnp.floating) else t)(jnp.asarray(a)))
    def _A_setup():
        B, Sq, D = 16, 144, 448
        Hq, Hkv, Sk, Dh = 16, 8, 1024, 256
        assert Hq % Hkv == 0, (Hq, Hkv)
        return {
            "x": _w((lambda *s: _rng.normal(s) * 0.8)(B, Sq, D)),
            "k_cache": _w((lambda *s: _rng.normal(s) * 0.8)(B, Hkv, Sk, Dh)),
            "v_cache": _w((lambda *s: _rng.normal(s) * 0.05)(B, Hkv, Sk, Dh)),
            "wq": _w((lambda *s: _rng.normal(s) * 0.8)(D, Hq * Dh) * (D ** -0.5)),
            "wo": _w((lambda *s: _rng.normal(s) * 0.05)(Hq * Dh, D) * ((Hq * Dh) ** -0.5)),
        }
    _A_in = _A_setup()

    def _B_setup():
        B, Sq, D = 16, 144, 448
        Hq, Hkv, Sk, Dh = 16, 8, 1024, 256
        assert Hq % Hkv == 0, (Hq, Hkv)
        return {
            "x": _w((lambda *s: _rng.normal(s) * 0.8)(B, Sq, D)),
            "k_cache": _w((lambda *s: _rng.normal(s) * 0.8)(B, Hkv, Sk, Dh)),
            "v_cache": _w((lambda *s: _rng.normal(s) * 0.05)(B, Hkv, Sk, Dh)),
            "wq": _w((lambda *s: _rng.normal(s) * 0.8)(D, Hq * Dh) * (D ** -0.5)),
            "wo": _w((lambda *s: _rng.normal(s) * 0.05)(Hq * Dh, D) * ((Hq * Dh) ** -0.5)),
        }
    _B_in = _B_setup()

    return {
        "A_x": _A_in["x"],
        "A_k_cache": _A_in["k_cache"],
        "A_v_cache": _A_in["v_cache"],
        "A_wq": _A_in["wq"],
        "A_wo": _A_in["wo"],
        "B_x": _B_in["x"],
        "B_k_cache": _B_in["k_cache"],
        "B_v_cache": _B_in["v_cache"],
        "B_wq": _B_in["wq"],
        "B_wo": _B_in["wo"],
    }

def reference(A_x, A_k_cache, A_v_cache, A_wq, A_wo, B_x, B_k_cache, B_v_cache, B_wq, B_wo):
    def _A_ref(x, k_cache, v_cache, wq, wo):
        B, Sq, D = x.shape
        Hq, Dh = 16, 256
        Hkv = k_cache.shape[1]
        rep = Hq // Hkv
        q = (lambda x, *d: x.transpose(*d))((x @ wq).reshape(B, Sq, Hq, Dh), 0, 2, 1, 3)
        k = jnp.repeat(k_cache, rep, axis=1)
        v = jnp.repeat(v_cache, rep, axis=1)
        scores = jnp.einsum("bhqd,bhkd->bhqk", q, k) * (Dh ** -0.5)
        p = _softmax(scores, axis=-1)
        o = jnp.einsum("bhqk,bhkd->bhqd", p, v)
        return (lambda x, *d: x.transpose(*d))(o, 0, 2, 1, 3).reshape(B, Sq, Hq * Dh) @ wo

    def _B_ref(x, k_cache, v_cache, wq, wo):
        B, Sq, D = x.shape
        Hq, Dh = 16, 256
        Hkv = k_cache.shape[1]
        rep = Hq // Hkv
        q = (lambda x, *d: x.transpose(*d))((x @ wq).reshape(B, Sq, Hq, Dh), 0, 2, 1, 3)
        k = jnp.repeat(k_cache, rep, axis=1)
        v = jnp.repeat(v_cache, rep, axis=1)
        scores = jnp.einsum("bhqd,bhkd->bhqk", q, k) * (Dh ** -0.5)
        p = _softmax(scores, axis=-1)
        o = jnp.einsum("bhqk,bhkd->bhqd", p, v)
        return (lambda x, *d: x.transpose(*d))(o, 0, 2, 1, 3).reshape(B, Sq, Hq * Dh) @ wo

    a = _A_ref(A_x, A_k_cache, A_v_cache, A_wq, A_wo)
    b = _B_ref(B_x, B_k_cache, B_v_cache, B_wq, B_wo)
    return jnp.concatenate([a, b], axis=-1)
```

```python
import functools
import jax
import jax.numpy as jnp
from jax import lax
import jax.experimental.pallas as pl
import jax.experimental.pallas.tpu as pltpu

LOG2E = 1.4426950408889634
NT = (((1,), (1,)), ((), ()))

B, Sq, D = 16, 144, 448
Hkv, Sk, Dh = 8, 1024, 256
NB = 8
T = NB * Sq
NTILE = T // 128
W = 2 * Dh
DM = 384
DR = D - DM

XO = {
    "A": "q0 q1 q2 q3 k0 k1 v0 k2 v1 o0 k3 v2 o1 k4 v3 o2 k5 v4 o3 k6 v5 o4 k7 v6 o5 v7 o6 o7 o8 n0",
    "B": "q0 k0 k1 v0 k2 v1 o0 k3 v2 o1 k4 v3 o2 k5 v4 o3 k6 v5 o4 q1 v6 k7 q2 o5 q3 v7 o6 o7 o8 n0",
}
YO = {
    "A": "k0 k1 v0 k2 v1 o0 k3 v2 o1 k4 v3 o2 d0 k5 v4 o3 k6 v5 o4 k7 v6 o5 d1 v7 o6 o7 o8 d2",
}


def make(nobc=True, xorder="B", yorder="A", LOOK=5):
    scale = (Dh ** -0.5) * LOG2E
    f32 = jnp.float32
    bf = jnp.bfloat16

    def kernel(xa, ka, va, wqa, wota, xb, kb, vb, wqb, wotb, out,
               x_s, wq_s, wo_s, k_s, v_s, q_s, o_s, acc_s, mid_s, st_s,
               kv_sem, wq_sem, wo_sem, x_sem, out_sem):
        srcs = ((xa, ka, va, wqa, wota), (xb, kb, vb, wqb, wotb))

        def kv_copies(bs, i):
            g, h, slot = i >> 4, i & 7, i & 1
            _, k, v, _, _ = srcs[bs]
            return (pltpu.make_async_copy(k.at[pl.ds(g * NB, NB), h], k_s.at[slot], kv_sem.at[0, slot]),
                    pltpu.make_async_copy(v.at[pl.ds(g * NB, NB), h], v_s.at[slot], kv_sem.at[1, slot]))

        def wq_copy(bs, j):
            c = pl.multiple_of((j & 7) * W, W)
            return pltpu.make_async_copy(srcs[bs][3].at[:, pl.ds(c, W)], wq_s.at[j & 15], wq_sem.at[j & 7])

        def wo_copies(bs, i):
            c = pl.multiple_of((i & 7) * W, W)
            wot = srcs[bs][4]
            dst = wo_s.at[i & 15]
            sem = wo_sem.at[i & 1]
            if bs == 0:
                return (pltpu.make_async_copy(wot.at[:, pl.ds(c, W)], dst, sem),)
            return (pltpu.make_async_copy(wot.at[pl.ds(DR, DM), pl.ds(c, W)], dst.at[pl.ds(0, DM)], sem),
                    pltpu.make_async_copy(wot.at[pl.ds(0, DR), pl.ds(c, W)], dst.at[pl.ds(DM, DR)], sem))

        def x_copy(bs, p):
            r = pl.multiple_of((p >> 1) * T, T)
            return pltpu.make_async_copy(srcs[bs][0].at[pl.ds(r, T)], x_s.at[p], x_sem.at[p])

        def out_main_copy(p, n0, nn):
            r = pl.multiple_of((p >> 1) * T + n0 * 128, 128)
            c = pl.multiple_of((p & 1) * W, W)
            return pltpu.make_async_copy(st_s.at[p, pl.ds(n0 * 128, nn * 128), pl.ds(0, DM)],
                                         out.at[pl.ds(r, nn * 128), pl.ds(c, DM)], out_sem.at[0])

        def out_mid_copy(p, n0, nn):
            r = pl.multiple_of((p >> 1) * T + n0 * 128, 128)
            return pltpu.make_async_copy(st_s.at[p, pl.ds(n0 * 128, nn * 128), pl.ds(DM, 128)],
                                         out.at[pl.ds(r, nn * 128), pl.ds(DM, 128)], out_sem.at[1])

        def start_sel(cond, blk, fn):
            for bs in range(2):
                @pl.when(jnp.logical_and(cond, blk == bs))
                def _():
                    for c in fn(bs):
                        c.start()

        def wait_block_inputs(i):
            for c in kv_copies(0, i):
                c.wait()
            @pl.when(i < 16)
            def _():
                wo_copies(0, i)[0].wait()

        def start_next_block(i):
            n = jnp.minimum(i + 1, 31)
            blkn = (n >> 3) & 1
            start_sel(i < 31, blkn, lambda bs: kv_copies(bs, n))
            start_sel(i < 15, blkn, lambda bs: wo_copies(bs, n))

        def wait_q_inputs(j):
            @pl.when(j < 16)
            def _():
                wq_copy(0, j).wait()
            @pl.when((j & 7) == 0)
            def _():
                x_copy(0, j >> 3).wait()

        def start_q_inputs(jn):
            n = jnp.minimum(jn, 31)
            blkn = (n >> 3) & 1
            start_sel(jn < 16, blkn, lambda bs: (wq_copy(bs, n),))
            start_sel(jnp.logical_and(jn < 32, (n & 7) == 0), blkn, lambda bs: (x_copy(bs, n >> 3),))

        def qproj_piece(j, n):
            x = x_s[j >> 3]
            w = wq_s[j & 15, :, n * 128:(n + 1) * 128]
            q = (jnp.dot(x, w, preferred_element_type=f32) * scale).astype(bf)
            r0 = (n // 2) * Sq
            c0 = (n % 2) * 128
            q_s[j & 7, :, r0:r0 + Sq, c0:c0 + 128] = q.reshape(NB, Sq, 128)

        def block(i, final):
            slot = i & 1
            p = i >> 3
            blk = p & 1
            h = i & 7
            j = i + LOOK - p
            wait_block_inputs(i)
            if not final:
                wait_q_inputs(j)
            start_next_block(i)

            def qk(b):
                s = lax.dot_general(q_s[i & 7, b], k_s[slot, b], NT, preferred_element_type=f32)
                m = jnp.max(s, axis=-1, keepdims=True)
                pb = jnp.exp2(s - m).astype(bf)
                pf = pb.astype(f32)
                lp = pf[:, 0:128]
                for c in range(1, Sk // 128):
                    lp = lp + pf[:, c * 128:(c + 1) * 128]
                return pb, lp

            def pv(b, pb, lp):
                o = jnp.dot(pb, v_s[slot, b], preferred_element_type=f32)
                lp = jnp.where(i >= 0, lp, o[:, 0:128])
                l = jnp.sum(lp, axis=-1, keepdims=True)
                r = pl.reciprocal(l, approx=True)
                r = r * (2.0 - l * r)
                o = (o * r).astype(bf)
                o_s[b * Sq:(b + 1) * Sq, :Dh] = o[:Sq]
                o_s[b * Sq:(b + 1) * Sq, Dh:] = o[Sq:]

            def oproj(n):
                cs = slice(n * 128, (n + 1) * 128)
                part = lax.dot_general(wo_s[i & 15], o_s[cs, :], NT, preferred_element_type=f32)
                if not final:
                    acc_s[blk, :, cs] = jnp.where(h == 0, 0.0, acc_s[blk, :, cs]) + part
                else:
                    fin = acc_s[blk, :, cs] + part
                    if LOOK > 4:
                        acc_s[blk, :, cs] = fin
                    r = fin[DM:]
                    ra = jnp.where(blk == 0, r, mid_s[:, cs])
                    mid_s[:, cs] = ra
                    z = jnp.concatenate([fin[:DM], ra, r], axis=0)
                    st_s[p, cs, :] = z.T.astype(bf)

            def outdma(n0, nn):
                @pl.when(h == 7)
                def _():
                    out_main_copy(p, n0, nn).start()
                @pl.when(jnp.logical_and(h == 7, blk == 1))
                def _():
                    out_mid_copy(p, n0, nn).start()

            S = {}
            order = (YO.get(yorder, yorder) if final else XO.get(xorder, xorder))
            for tok in order.split():
                kind, n = tok[0], int(tok[1:])
                if kind == "k":
                    S[n] = qk(n)
                elif kind == "v":
                    pv(n, *S.pop(n))
                elif kind == "o":
                    oproj(n)
                elif kind == "q":
                    qproj_piece(j, n)
                elif kind == "n":
                    start_q_inputs(j + 2)
                elif kind == "d":
                    outdma(3 * n, 3)

        x_copy(0, 0).start()
        wq_copy(0, 0).start()
        wq_copy(0, 1).start()
        x_copy(0, 0).wait()
        for c in kv_copies(0, 0) + wo_copies(0, 0):
            c.start()

        def pro(j, c):
            wq_copy(0, j).wait()
            wq_copy(0, j + 2).start()
            for n in range(4):
                qproj_piece(j, n)
            return c
        lax.fori_loop(0, LOOK, pro, 0)

        def phase(p, c):
            nx = jnp.where(p == 3, 8 - (LOOK - 3), 7)
            def xb_(h, c2):
                block(p * 8 + h, False)
                return c2
            lax.fori_loop(0, nx, xb_, 0)
            def yb_(h, c2):
                block(p * 8 + h, True)
                return c2
            lax.fori_loop(nx, 8, yb_, 0)
            return c
        lax.fori_loop(0, 4, phase, 0)

        for p in range(4):
            out_main_copy(p, 0, NTILE).wait()
        for p in (1, 3):
            out_mid_copy(p, 0, NTILE).wait()

    @jax.jit
    def f(A_x, A_k_cache, A_v_cache, A_wq, A_wo, B_x, B_k_cache, B_v_cache, B_wq, B_wo):
        any_spec = pl.BlockSpec(memory_space=pl.ANY)
        out = pl.pallas_call(
            kernel,
            in_specs=[any_spec] * 10,
            out_specs=any_spec,
            out_shape=jax.ShapeDtypeStruct((B * Sq, 2 * D), bf),
            scratch_shapes=[
                pltpu.VMEM((4, T, D), bf),
                pltpu.VMEM((16, D, W), bf),
                pltpu.VMEM((16, D, W), bf),
                pltpu.VMEM((2, NB, Sk, Dh), bf),
                pltpu.VMEM((2, NB, Sk, Dh), bf),
                pltpu.VMEM((8, NB, 2 * Sq, Dh), bf),
                pltpu.VMEM((T, W), bf),
                pltpu.VMEM((2, D, T), f32),
                pltpu.VMEM((DR, T), f32),
                pltpu.VMEM((4, T, W), bf),
                pltpu.SemaphoreType.DMA((2, 2)),
                pltpu.SemaphoreType.DMA((8,)),
                pltpu.SemaphoreType.DMA((2,)),
                pltpu.SemaphoreType.DMA((4,)),
                pltpu.SemaphoreType.DMA((2,)),
            ],
            compiler_params=pltpu.CompilerParams(
                disable_bounds_checks=nobc,
                vmem_limit_bytes=100 * 1024 * 1024),
        )(A_x.reshape(B * Sq, D), A_k_cache, A_v_cache, A_wq, A_wo.T, B_x.reshape(B * Sq, D), B_k_cache, B_v_cache, B_wq, B_wo.T)
        return out.reshape(B, Sq, 2 * D)
    return f

pallas_concat_heads__gqa_block_cached__gqa_block_cached__near_ridge_kernel = make(LOOK=4)
```

```python
import jax
import jax.numpy as jnp
from jax import lax
import jax.experimental.pallas as pl
import jax.experimental.pallas.tpu as pltpu

LOG2E = 1.4426950408889634
NT = (((1,), (1,)), ((), ()))

B, SQ, D = 16, 144, 448
HKV, SK, DH = 8, 1024, 256
NB = 8
T = NB * SQ
NTILE = T // 128
W = 2 * DH
DM = 384
DR = D - DM
LOOK = 5
NBLK = 32

X_ORDER = ("q0 k0 k1 v0 k2 v1 o0 k3 v2 o1 k4 v3 o2 k5 v4 o3 k6 v5 o4 k7 v6 o5 "
           "q1 v7 q2 o6 o7 o8 q3 n0")
Y_ORDER = ("k0 k1 v0 k2 v1 o0 t0 k3 v2 o1 t1 k4 v3 o2 t2 k5 v4 o3 t3 k6 v5 o4 "
           "t4 k7 v6 o5 t5 v7 o6 t6 o7 t7 o8 t8")

F32 = jnp.float32
BF16 = jnp.bfloat16
SCALE = (DH ** -0.5) * LOG2E


def _kernel(xa, ka, va, wqa, wota, xb, kb, vb, wqb, wotb, out,
            x_s, wq_s, wo_s, k_s, v_s, q_s, o_s, acc_s, mid_s, st_s,
            kv_sem, wq_sem, wo_sem, x_sem, out_sem, bar_sem):
    srcs = ((xa, ka, va, wqa, wota), (xb, kb, vb, wqb, wotb))
    copy = pltpu.make_async_copy

    def wait_for(dst, sem):
        copy(dst, dst, sem).wait()

    def kv_copies(ab, i):
        g, h, slot = i >> 4, i & 7, i & 1
        return (copy(srcs[ab][1].at[pl.ds(g * NB, NB), h], k_s.at[slot], kv_sem.at[0, slot]),
                copy(srcs[ab][2].at[pl.ds(g * NB, NB), h], v_s.at[slot], kv_sem.at[1, slot]))

    def wq_copy(ab, j):
        c = pl.multiple_of((j & 7) * W, W)
        return copy(srcs[ab][3].at[:, pl.ds(c, W)], wq_s.at[j & 15], wq_sem.at[j & 7])

    def wo_copies(ab, i):
        c = pl.multiple_of((i & 7) * W, W)
        wot, dst, sem = srcs[ab][4], wo_s.at[i & 15], wo_sem.at[i & 1]
        if ab == 0:
            return (copy(wot.at[:, pl.ds(c, W)], dst, sem),)
        return (copy(wot.at[pl.ds(DR, DM), pl.ds(c, W)], dst.at[pl.ds(0, DM)], sem),
                copy(wot.at[pl.ds(0, DR), pl.ds(c, W)], dst.at[pl.ds(DM, DR)], sem))

    def x_copy(ab, p):
        r = pl.multiple_of((p >> 1) * T, T)
        return copy(srcs[ab][0].at[pl.ds(r, T)], x_s.at[p], x_sem.at[p])

    def start_from(cond, ab_dyn, fn):
        for ab in range(2):
            @pl.when(jnp.logical_and(cond, ab_dyn == ab))
            def _():
                for c in fn(ab):
                    c.start()

    def qproj_piece(j, n):
        w = wq_s[j & 15, :, n * 128:(n + 1) * 128]
        q = (jnp.dot(x_s[j >> 3], w, preferred_element_type=F32) * SCALE).astype(BF16)
        r0, c0 = (n // 2) * SQ, (n % 2) * 128
        q_s[j & 7, :, r0:r0 + SQ, c0:c0 + 128] = q.reshape(NB, SQ, 128)

    def block(i, final):
        slot, p, h = i & 1, i >> 3, i & 7
        ab = p & 1
        j = i + LOOK - p

        wait_for(k_s.at[slot], kv_sem.at[0, slot])
        wait_for(v_s.at[slot], kv_sem.at[1, slot])

        @pl.when(i < 16)
        def _():
            wait_for(wo_s.at[i & 15], wo_sem.at[i & 1])
        if not final:
            @pl.when(j < 16)
            def _():
                wait_for(wq_s.at[j & 15], wq_sem.at[j & 7])

            @pl.when((j & 7) == 0)
            def _():
                wait_for(x_s.at[j >> 3], x_sem.at[j >> 3])

        nxt = jnp.minimum(i + 1, NBLK - 1)
        start_from(i < NBLK - 1, (nxt >> 3) & 1, lambda a: kv_copies(a, nxt))
        start_from(i < 15, (nxt >> 3) & 1, lambda a: wo_copies(a, nxt))

        always = i >= 0
        staged = []

        def qk(b):
            s = lax.dot_general(q_s[i & 7, b], k_s[slot, b], NT, preferred_element_type=F32)
            m = jnp.max(s, axis=-1, keepdims=True)
            pb = jnp.exp2(s - m).astype(BF16)
            pf = pb.astype(F32)
            lp = pf[:, 0:128]
            for c in range(1, SK // 128):
                lp = lp + pf[:, c * 128:(c + 1) * 128]
            return pb, lp

        def pv(b, pb, lp):
            o = jnp.dot(pb, v_s[slot, b], preferred_element_type=F32)
            lp = jnp.where(always, lp, o[:, 0:128])
            if staged:
                zt = staged.pop()
                ls = [lp[:128], lp[128:256], lp[256:]]
                for c in range(4):
                    ls[c % 2] = jnp.where(always, ls[c % 2], zt[:, c * 128:(c + 1) * 128])
                lp = jnp.concatenate(ls, axis=0)
            l = jnp.sum(lp, axis=-1, keepdims=True)
            r = pl.reciprocal(l, approx=True)
            r = r * (2.0 - l * r)
            o = (o * r).astype(BF16)
            o_s[b * SQ:(b + 1) * SQ, :DH] = o[:SQ]
            o_s[b * SQ:(b + 1) * SQ, DH:] = o[SQ:]

        def oproj(n):
            cs = slice(n * 128, (n + 1) * 128)
            part = lax.dot_general(wo_s[i & 15], o_s[cs, :], NT, preferred_element_type=F32)
            if not final:
                acc_s[ab, :, cs] = jnp.where(h == 0, 0.0, acc_s[ab, :, cs]) + part
            else:
                fin = acc_s[ab, :, cs] + part
                acc_s[ab, :, cs] = fin
                r = fin[DM:]
                ra = jnp.where(ab == 0, r, mid_s[:, cs])
                mid_s[:, cs] = ra
                zt = jnp.concatenate([fin[:DM], ra, r], axis=0).T
                st_s[p, cs, :] = zt.astype(BF16)
                staged.append(zt)

        def write_back(n):
            r = pl.multiple_of((p >> 1) * T + n * 128, 128)
            c = pl.multiple_of(ab * W, W)

            @pl.when(h == HKV - 1)
            def _():
                copy(st_s.at[p, pl.ds(n * 128, 128), pl.ds(0, DM)],
                     out.at[pl.ds(r, 128), pl.ds(c, DM)], out_sem.at[0]).start()

            @pl.when(jnp.logical_and(h == HKV - 1, ab == 1))
            def _():
                copy(st_s.at[p, pl.ds(n * 128, 128), pl.ds(DM, 128)],
                     out.at[pl.ds(r, 128), pl.ds(DM, 128)], out_sem.at[1]).start()

        def prefetch_q_operands(jn):
            n = jnp.minimum(jn, NBLK - 1)
            start_from(jn < 16, (n >> 3) & 1, lambda a: (wq_copy(a, n),))
            start_from(jnp.logical_and(jn < NBLK, (n & 7) == 0), (n >> 3) & 1,
                       lambda a: (x_copy(a, n >> 3),))

        live = {}
        for tok in (Y_ORDER if final else X_ORDER).split():
            kind, n = tok[0], int(tok[1:])
            if kind == "k":
                live[n] = qk(n)
            elif kind == "v":
                pv(n, *live.pop(n))
            elif kind == "o":
                oproj(n)
            elif kind == "q":
                qproj_piece(j, n)
            elif kind == "t":
                write_back(n)
            else:
                prefetch_q_operands(j + 2)

    def fence():
        pl.semaphore_signal(bar_sem, 1)
        pl.semaphore_wait(bar_sem, 1)

    half = T // 2
    xh = [copy(xa.at[pl.ds(c * half, half)], x_s.at[0, pl.ds(c * half, half)], x_sem.at[c])
          for c in range(2)]
    wh = [copy(wqa.at[:, pl.ds(c * DH, DH)], wq_s.at[0, :, pl.ds(c * DH, DH)], wq_sem.at[7 * c])
          for c in range(2)]
    for c in range(2):
        xh[c].start()
        wh[c].start()
        fence()
    for j in range(1, LOOK):
        wq_copy(0, j).start()
    fence()
    for c in kv_copies(0, 0) + wo_copies(0, 0) + (wq_copy(0, LOOK),):
        c.start()
    fence()
    wq_copy(0, LOOK + 1).start()

    def qproj0(rh, ch):
        x = x_s[0, rh * half:(rh + 1) * half]
        w = wq_s[0, :, ch * DH:(ch + 1) * DH]
        q = (jnp.dot(x, w, preferred_element_type=F32) * SCALE).astype(BF16)
        q_s[0, rh * (NB // 2):(rh + 1) * (NB // 2), ch * SQ:(ch + 1) * SQ, :] = (
            q.reshape(NB // 2, SQ, DH))

    xh[0].wait()
    wh[0].wait()
    qproj0(0, 0)
    xh[1].wait()
    wh[1].wait()
    qproj0(0, 1)
    qproj0(1, 0)
    qproj0(1, 1)

    def qproj_pair(jj, carry):
        j = 1 + 2 * jj
        wq_copy(0, j).wait()
        wq_copy(0, j + 1).wait()
        for jn in (j, j + 1):
            for n in range(4):
                qproj_piece(jn, n)
        return carry
    lax.fori_loop(0, (LOOK - 1) // 2, qproj_pair, 0)

    def phase(p, carry):
        nx = jnp.where(p == 3, HKV - (LOOK - 3), HKV - 1)

        def x_body(h, c):
            block(p * HKV + h, False)
            return c
        lax.fori_loop(0, nx, x_body, 0)

        def y_body(h, c):
            block(p * HKV + h, True)
            return c
        lax.fori_loop(nx, HKV, y_body, 0)
        return carry
    lax.fori_loop(0, 4, phase, 0)

    wait_for(st_s.at[:, :, pl.ds(0, DM)], out_sem.at[0])
    wait_for(st_s.at[pl.ds(0, 2), :, pl.ds(DM, 128)], out_sem.at[1])


@jax.jit
def pallas_concat_heads__gqa_block_cached__gqa_block_cached__near_ridge_kernel(
    A_x: jax.Array,
    A_k_cache: jax.Array,
    A_v_cache: jax.Array,
    A_wq: jax.Array,
    A_wo: jax.Array,
    B_x: jax.Array,
    B_k_cache: jax.Array,
    B_v_cache: jax.Array,
    B_wq: jax.Array,
    B_wo: jax.Array,
):
    assert A_x.shape == (B, SQ, D) and A_k_cache.shape == (B, HKV, SK, DH)
    any_spec = pl.BlockSpec(memory_space=pl.ANY)
    out = pl.pallas_call(
        _kernel,
        in_specs=[any_spec] * 10,
        out_specs=any_spec,
        out_shape=jax.ShapeDtypeStruct((B * SQ, 2 * D), BF16),
        scratch_shapes=[
            pltpu.VMEM((4, T, D), BF16),
            pltpu.VMEM((16, D, W), BF16),
            pltpu.VMEM((16, D, W), BF16),
            pltpu.VMEM((2, NB, SK, DH), BF16),
            pltpu.VMEM((2, NB, SK, DH), BF16),
            pltpu.VMEM((8, NB, 2 * SQ, DH), BF16),
            pltpu.VMEM((T, W), BF16),
            pltpu.VMEM((2, D, T), F32),
            pltpu.VMEM((DR, T), F32),
            pltpu.VMEM((4, T, W), BF16),
            pltpu.SemaphoreType.DMA((2, 2)),
            pltpu.SemaphoreType.DMA((8,)),
            pltpu.SemaphoreType.DMA((2,)),
            pltpu.SemaphoreType.DMA((4,)),
            pltpu.SemaphoreType.DMA((2,)),
            pltpu.SemaphoreType.REGULAR,
        ],
        compiler_params=pltpu.CompilerParams(
            disable_bounds_checks=True,
            vmem_limit_bytes=100 * 1024 * 1024),
    )(A_x.reshape(B * SQ, D), A_k_cache, A_v_cache, A_wq, A_wo.T,
      B_x.reshape(B * SQ, D), B_k_cache, B_v_cache, B_wq, B_wo.T)
    return out.reshape(B, SQ, 2 * D)
```

```python
import jax
import jax.numpy as jnp
from jax import lax
import jax.experimental.pallas as pl
import jax.experimental.pallas.tpu as pltpu

LOG2E = 1.4426950408889634
NT = (((1,), (1,)), ((), ()))

B, SQ, D = 16, 144, 448
HKV, SK, DH = 8, 1024, 256
NB = 8
T = NB * SQ
NTILE = T // 128
W = 2 * DH
DM = 384
DR = D - DM
LOOK = 5
NBLK = 32

X_ORDER = ("q0 k0 k1 v0 k2 v1 o0 k3 v2 o1 k4 v3 o2 k5 v4 o3 k6 v5 o4 k7 v6 o5 "
           "q1 v7 q2 o6 o7 o8 q3 n0")
Y_ORDER = ("k0 k1 v0 k2 v1 o0 t0 k3 v2 o1 t1 k4 v3 o2 t2 k5 v4 o3 t3 k6 v5 o4 "
           "t4 k7 v6 o5 t5 v7 o6 t6 o7 t7 o8 t8")

F32 = jnp.float32
BF16 = jnp.bfloat16
SCALE = (DH ** -0.5) * LOG2E


def _kernel(xa, ka, va, wqa, wota, xb, kb, vb, wqb, wotb, out,
            x_s, wq_s, wo_s, k_s, v_s, q_s, o_s, acc_s, mid_s, st_s,
            kv_sem, wq_sem, wo_sem, x_sem, out_sem, bar_sem):
    srcs = ((xa, ka, va, wqa, wota), (xb, kb, vb, wqb, wotb))
    copy = pltpu.make_async_copy

    def wait_for(dst, sem):
        copy(dst, dst, sem).wait()

    def kv_copies(ab, i):
        g, h, slot = i >> 4, i & 7, i & 1
        return (copy(srcs[ab][1].at[pl.ds(g * NB, NB), h], k_s.at[slot], kv_sem.at[0, slot]),
                copy(srcs[ab][2].at[pl.ds(g * NB, NB), h], v_s.at[slot], kv_sem.at[1, slot]))

    def wq_copy(ab, j):
        c = pl.multiple_of((j & 7) * W, W)
        return copy(srcs[ab][3].at[:, pl.ds(c, W)], wq_s.at[j & 15], wq_sem.at[j & 7])

    def wo_copies(ab, i):
        c = pl.multiple_of((i & 7) * W, W)
        wot, dst, sem = srcs[ab][4], wo_s.at[i & 15], wo_sem.at[i & 1]
        if ab == 1:
            return (copy(wot.at[:, pl.ds(c, W)], dst, sem),)
        return (copy(wot.at[pl.ds(DM, DR), pl.ds(c, W)], dst.at[pl.ds(0, DR)], sem),
                copy(wot.at[pl.ds(0, DM), pl.ds(c, W)], dst.at[pl.ds(DR, DM)], sem))

    def x_copy(ab, p):
        r = pl.multiple_of((p >> 1) * T, T)
        return copy(srcs[ab][0].at[pl.ds(r, T)], x_s.at[p], x_sem.at[p])

    def start_from(cond, ab_dyn, fn):
        for ab in range(2):
            @pl.when(jnp.logical_and(cond, ab_dyn == ab))
            def _():
                for c in fn(ab):
                    c.start()

    def qproj_piece(j, n):
        w = wq_s[j & 15, :, n * 128:(n + 1) * 128]
        q = (jnp.dot(x_s[j >> 3], w, preferred_element_type=F32) * SCALE).astype(BF16)
        r0, c0 = (n // 2) * SQ, (n % 2) * 128
        q_s[j & 7, :, r0:r0 + SQ, c0:c0 + 128] = q.reshape(NB, SQ, 128)

    def block(i, final):
        slot, p, h = i & 1, i >> 3, i & 7
        ab = p & 1
        j = i + LOOK - p

        wait_for(k_s.at[slot], kv_sem.at[0, slot])
        wait_for(v_s.at[slot], kv_sem.at[1, slot])

        @pl.when(i < 16)
        def _():
            wait_for(wo_s.at[i & 15], wo_sem.at[i & 1])
        if not final:
            @pl.when(j < 16)
            def _():
                wait_for(wq_s.at[j & 15], wq_sem.at[j & 7])

            @pl.when((j & 7) == 0)
            def _():
                wait_for(x_s.at[j >> 3], x_sem.at[j >> 3])

        nxt = jnp.minimum(i + 1, NBLK - 1)
        start_from(i < NBLK - 1, (nxt >> 3) & 1, lambda a: kv_copies(a, nxt))
        start_from(i < 15, (nxt >> 3) & 1, lambda a: wo_copies(a, nxt))

        always = i >= 0
        staged = []

        def qk(b):
            s = lax.dot_general(q_s[i & 7, b], k_s[slot, b], NT, preferred_element_type=F32)
            m = jnp.max(s, axis=-1, keepdims=True)
            pb = jnp.exp2(s - m).astype(BF16)
            pf = pb.astype(F32)
            lp = pf[:, 0:128]
            for c in range(1, SK // 128):
                lp = lp + pf[:, c * 128:(c + 1) * 128]
            return pb, lp

        def pv(b, pb, lp):
            o = jnp.dot(pb, v_s[slot, b], preferred_element_type=F32)
            lp = jnp.where(always, lp, o[:, 0:128])
            if staged:
                zt = staged.pop()
                ls = [lp[:128], lp[128:256], lp[256:]]
                for c in range(4):
                    ls[c % 2] = jnp.where(always, ls[c % 2], zt[:, c * 128:(c + 1) * 128])
                lp = jnp.concatenate(ls, axis=0)
            l = jnp.sum(lp, axis=-1, keepdims=True)
            r = pl.reciprocal(l, approx=True)
            r = r * (2.0 - l * r)
            o = (o * r).astype(BF16)
            o_s[b * SQ:(b + 1) * SQ, :DH] = o[:SQ]
            o_s[b * SQ:(b + 1) * SQ, DH:] = o[SQ:]

        def oproj(n):
            cs = slice(n * 128, (n + 1) * 128)
            part = lax.dot_general(wo_s[i & 15], o_s[cs, :], NT, preferred_element_type=F32)
            if not final:
                acc_s[ab, :, cs] = jnp.where(h == 0, 0.0, acc_s[ab, :, cs]) + part
            else:
                fin = acc_s[ab, :, cs] + part
                acc_s[ab, :, cs] = fin
                r = fin[:DR]
                ra = jnp.where(ab == 0, r, mid_s[:, cs])
                mid_s[:, cs] = ra
                zt = jnp.concatenate([fin[DR:], ra, r], axis=0).T
                st_s[p, cs, :] = zt.astype(BF16)
                staged.append(zt)

        def write_back(n):
            r = pl.multiple_of((p >> 1) * T + n * 128, 128)
            c = pl.multiple_of(ab * W, W)

            @pl.when(h == HKV - 1)
            def _():
                copy(st_s.at[p, pl.ds(n * 128, 128), pl.ds(0, DM)],
                     out.at[pl.ds(r, 128), pl.ds(c, DM)], out_sem.at[0]).start()

            @pl.when(jnp.logical_and(h == HKV - 1, ab == 1))
            def _():
                copy(st_s.at[p, pl.ds(n * 128, 128), pl.ds(DM, 128)],
                     out.at[pl.ds(r, 128), pl.ds(DM, 128)], out_sem.at[1]).start()

        def prefetch_q_operands(jn):
            n = jnp.minimum(jn, NBLK - 1)
            start_from(jn < 16, (n >> 3) & 1, lambda a: (wq_copy(a, n),))
            start_from(jnp.logical_and(jn < NBLK, (n & 7) == 0), (n >> 3) & 1,
                       lambda a: (x_copy(a, n >> 3),))

        live = {}
        for tok in (Y_ORDER if final else X_ORDER).split():
            kind, n = tok[0], int(tok[1:])
            if kind == "k":
                live[n] = qk(n)
            elif kind == "v":
                pv(n, *live.pop(n))
            elif kind == "o":
                oproj(n)
            elif kind == "q":
                qproj_piece(j, n)
            elif kind == "t":
                write_back(n)
            else:
                prefetch_q_operands(j + 2)

    def fence():
        pl.semaphore_signal(bar_sem, 1)
        pl.semaphore_wait(bar_sem, 1)

    half = T // 2
    xh = [copy(xa.at[pl.ds(c * half, half)], x_s.at[0, pl.ds(c * half, half)], x_sem.at[c])
          for c in range(2)]
    wh = [copy(wqa.at[:, pl.ds(c * DH, DH)], wq_s.at[0, :, pl.ds(c * DH, DH)], wq_sem.at[7 * c])
          for c in range(2)]
    for c in range(2):
        xh[c].start()
        wh[c].start()
        fence()
    for j in range(1, LOOK):
        wq_copy(0, j).start()
    fence()
    for c in kv_copies(0, 0) + wo_copies(0, 0) + (wq_copy(0, LOOK),):
        c.start()
    fence()
    wq_copy(0, LOOK + 1).start()

    def qproj0(rh, ch):
        x = x_s[0, rh * half:(rh + 1) * half]
        w = wq_s[0, :, ch * DH:(ch + 1) * DH]
        q = (jnp.dot(x, w, preferred_element_type=F32) * SCALE).astype(BF16)
        q_s[0, rh * (NB // 2):(rh + 1) * (NB // 2), ch * SQ:(ch + 1) * SQ, :] = (
            q.reshape(NB // 2, SQ, DH))

    xh[0].wait()
    wh[0].wait()
    qproj0(0, 0)
    xh[1].wait()
    wh[1].wait()
    qproj0(0, 1)
    qproj0(1, 0)
    qproj0(1, 1)

    def qproj_pair(jj, carry):
        j = 1 + 2 * jj
        wq_copy(0, j).wait()
        wq_copy(0, j + 1).wait()
        for jn in (j, j + 1):
            for n in range(4):
                qproj_piece(jn, n)
        return carry
    lax.fori_loop(0, (LOOK - 1) // 2, qproj_pair, 0)

    def phase(p, carry):
        nx = jnp.where(p == 3, HKV - (LOOK - 3), HKV - 1)

        def x_body(h, c):
            block(p * HKV + h, False)
            return c
        lax.fori_loop(0, nx, x_body, 0)

        def y_body(h, c):
            block(p * HKV + h, True)
            return c
        lax.fori_loop(nx, HKV, y_body, 0)
        return carry
    lax.fori_loop(0, 4, phase, 0)

    wait_for(st_s.at[:, :, pl.ds(0, DM)], out_sem.at[0])
    wait_for(st_s.at[pl.ds(0, 2), :, pl.ds(DM, 128)], out_sem.at[1])


@jax.jit
def pallas_concat_heads__gqa_block_cached__gqa_block_cached__near_ridge_kernel(
    A_x: jax.Array,
    A_k_cache: jax.Array,
    A_v_cache: jax.Array,
    A_wq: jax.Array,
    A_wo: jax.Array,
    B_x: jax.Array,
    B_k_cache: jax.Array,
    B_v_cache: jax.Array,
    B_wq: jax.Array,
    B_wo: jax.Array,
):
    assert A_x.shape == (B, SQ, D) and A_k_cache.shape == (B, HKV, SK, DH)
    any_spec = pl.BlockSpec(memory_space=pl.ANY)
    out = pl.pallas_call(
        _kernel,
        in_specs=[any_spec] * 10,
        out_specs=any_spec,
        out_shape=jax.ShapeDtypeStruct((B * SQ, 2 * D), BF16),
        scratch_shapes=[
            pltpu.VMEM((4, T, D), BF16),
            pltpu.VMEM((16, D, W), BF16),
            pltpu.VMEM((16, D, W), BF16),
            pltpu.VMEM((2, NB, SK, DH), BF16),
            pltpu.VMEM((2, NB, SK, DH), BF16),
            pltpu.VMEM((8, NB, 2 * SQ, DH), BF16),
            pltpu.VMEM((T, W), BF16),
            pltpu.VMEM((2, D, T), F32),
            pltpu.VMEM((DR, T), F32),
            pltpu.VMEM((4, T, W), BF16),
            pltpu.SemaphoreType.DMA((2, 2)),
            pltpu.SemaphoreType.DMA((8,)),
            pltpu.SemaphoreType.DMA((2,)),
            pltpu.SemaphoreType.DMA((4,)),
            pltpu.SemaphoreType.DMA((2,)),
            pltpu.SemaphoreType.REGULAR,
        ],
        compiler_params=pltpu.CompilerParams(
            disable_bounds_checks=True,
            vmem_limit_bytes=100 * 1024 * 1024),
    )(A_x.reshape(B * SQ, D), A_k_cache, A_v_cache, A_wq, A_wo.T,
      B_x.reshape(B * SQ, D), B_k_cache, B_v_cache, B_wq, B_wo.T)
    return out.reshape(B, SQ, 2 * D)
```

```python
import jax
import jax.numpy as jnp
from jax import lax
import jax.experimental.pallas as pl
import jax.experimental.pallas.tpu as pltpu

LOG2E = 1.4426950408889634
NT = (((1,), (1,)), ((), ()))

B, SQ, D = 16, 144, 448
HKV, SK, DH = 8, 1024, 256
NB = 8
T = NB * SQ
W = 2 * DH
DM = 384
DR = D - DM
LOOK = 5
NBLK = 32
NG = 27
R = NG * 16
KC = 8
NC = DR // KC

X_ORDER = ("r0 k0 k1 v0 k2 v1 o0 k3 v2 o1 k4 v3 o2 k5 v4 o3 k6 v5 o4 k7 r1 v6 o5 "
           "r2 v7 z0 o6 o7 o8 w0 r3 n0")
Y_ORDER = ("b0 k0 k1 v0 k2 v1 o0 t0 k3 v2 o1 t1 k4 v3 o2 t2 k5 v4 o3 t3 k6 v5 o4 "
           "t4 k7 v6 o5 t5 v7 o6 t6 o7 t7 o8 t8")

F32 = jnp.float32
BF16 = jnp.bfloat16
U32 = jnp.uint32
SCALE = (DH ** -0.5) * LOG2E


def _kernel(xa, ka, va, wqa, wota, xb, kb, vb, wqb, wotb, out,
            x_s, wq_s, wo_s, k_s, v_s, q_s, o_s, acc_s, mid_s, st_s, xt_s, xb_s, wb_s, wt_s,
            kv_sem, wq_sem, wo_sem, x_sem, out_sem, xt_sem, wt_sem, bar_sem):
    srcs = ((xa, ka, va, wqa, wota), (xb, kb, vb, wqb, wotb))
    copy = pltpu.make_async_copy

    def wait_for(dst, sem):
        copy(dst, dst, sem).wait()

    def kv_copies(ab, i):
        g, h, slot = i >> 4, i & 7, i & 1
        return (copy(srcs[ab][1].at[pl.ds(g * NB, NB), h], k_s.at[slot], kv_sem.at[0, slot]),
                copy(srcs[ab][2].at[pl.ds(g * NB, NB), h], v_s.at[slot], kv_sem.at[1, slot]))

    def wq_copy(ab, j):
        c = pl.multiple_of((j & 7) * W, W)
        return copy(srcs[ab][3].at[:, pl.ds(c, W)], wq_s.at[j & 15], wq_sem.at[j & 7])

    def wt_copy(ab, j):
        c = pl.multiple_of((j & 7) * W, W)
        return copy(srcs[ab][3].at[pl.ds(DM, DR), pl.ds(c, W)], wt_s.at[j & 15], wt_sem.at[j & 3])

    def wo_copies(ab, i):
        c = pl.multiple_of((i & 7) * W, W)
        wot, dst, sem = srcs[ab][4], wo_s.at[i & 15], wo_sem.at[i & 1]
        if ab == 1:
            return (copy(wot.at[:, pl.ds(c, W)], dst, sem),)
        return (copy(wot.at[pl.ds(DM, DR), pl.ds(c, W)], dst.at[pl.ds(0, DR)], sem),
                copy(wot.at[pl.ds(0, DM), pl.ds(c, W)], dst.at[pl.ds(DR, DM)], sem))

    def x_copy(ab, p):
        r = pl.multiple_of((p >> 1) * T, T)
        return copy(srcs[ab][0].at[pl.ds(r, T)], x_s.at[p], x_sem.at[p])

    def xt_copy(p):
        return copy(srcs[p & 1][0].at[pl.ds((p >> 1) * T, R), pl.ds(DM, DR)], xt_s.at[p],
                    xt_sem.at[min(p, 2)])

    def start_from(cond, ab_dyn, fn):
        for ab in range(2):
            @pl.when(jnp.logical_and(cond, ab_dyn == ab))
            def _():
                for c in fn(ab):
                    c.start()

    def store_q(j, q, row0, col0):
        nrow, ncol = q.shape
        cw = min(ncol, DH)
        for c0 in range(col0, col0 + ncol, cw):
            head, cc = c0 // DH, c0 % DH
            r = row0
            while r < row0 + nrow:
                b, off = r // SQ, r % SQ
                n = min(SQ - off, row0 + nrow - r)
                q_s[j & 7, b, head * SQ + off:head * SQ + off + n, cc:cc + cw] = (
                    q[r - row0:r - row0 + n, c0 - col0:c0 - col0 + cw])
                r += n

    def halves_on_lanes(bc, n):
        v = pltpu.bitcast(bc, BF16).astype(F32).reshape(n, 16, 128)
        return jnp.concatenate([v[:, :8], v[:, 8:]], axis=2)

    def build_xb(p, slot, g0, ng):
        if ng == NG:
            xt = pltpu.bitcast(xt_s[p], U32)
            x2 = jnp.concatenate([xt, xt], axis=1).reshape(NG, 1, 8, 128)
            src = jnp.broadcast_to(x2, (NG, DR, 8, 128)).reshape(NG * DR * 8, 128)
            idx = lax.broadcasted_iota(jnp.int32, (NG, DR, 8, 128), 1).reshape(NG * DR * 8, 128)
            bc = jnp.take_along_axis(src, idx, axis=1, mode="promise_in_bounds")
            xb_s[slot] = halves_on_lanes(bc, NG * DR).reshape(NG, DR, 8, 256)
        else:
            xt = pltpu.bitcast(xt_s[p, pl.ds(pl.multiple_of(g0 * 16, 16), ng * 16), :], U32)
            for k in range(DR):
                bc = jnp.broadcast_to(xt[:, k:k + 1], (ng * 8, 128))
                xb_s[slot, pl.ds(g0, ng), k] = halves_on_lanes(bc, ng)

    def build_wb(j, always, dep):
        w32 = wt_s[j & 15].astype(F32)
        step = dep.shape[0] // 256 * 8
        for c in range(4):
            dc = jnp.concatenate([dep[(c * 8 + r) * step:(c * 8 + r) * step + 8] for r in range(8)], axis=0)
            wc = jnp.where(always, w32[:, c * 128:(c + 1) * 128], dc)
            wb_s[:, c] = jnp.broadcast_to(wc[:, None, :], (DR, 8, 128)).reshape(NC, KC, 8, 128)

    def block(i, final):
        slot, p, h = i & 1, i >> 3, i & 7
        ab = p & 1
        j = i + LOOK - p
        jp = j >> 3

        wait_for(k_s.at[slot], kv_sem.at[0, slot])
        wait_for(v_s.at[slot], kv_sem.at[1, slot])

        @pl.when(i < 16)
        def _():
            wait_for(wo_s.at[i & 15], wo_sem.at[i & 1])
        if not final:
            @pl.when(j < 16)
            def _():
                wait_for(wq_s.at[j & 15], wq_sem.at[j & 7])

            @pl.when((j & 7) == 0)
            def _():
                wait_for(x_s.at[jp], x_sem.at[jp])

            @pl.when(j + 1 < LOOK + 16)
            def _():
                wait_for(wt_s.at[(j + 1) & 15], wt_sem.at[(j + 1) & 3])
        else:
            @pl.when(p == 0)
            def _():
                wait_for(xt_s.at[pl.ds(2, 2)], xt_sem.at[2])

        nxt = jnp.minimum(i + 1, NBLK - 1)
        start_from(i < NBLK - 1, (nxt >> 3) & 1, lambda a: kv_copies(a, nxt))
        start_from(i < 15, (nxt >> 3) & 1, lambda a: wo_copies(a, nxt))

        always = i >= 0
        staged = []

        groups = [] if final else list(range(NG))
        tails, queue, deps = [], [], []

        def tail_group():
            g = groups.pop(0)
            x = xb_s[jp & 1, g].reshape(NC, 1, KC, 8, 256)
            w = wb_s[...]
            pr = jnp.sum(x * jnp.concatenate([w, w], axis=4), axis=2).reshape(NC, 32, 256)
            cum = [pr[0]]
            for c in range(1, NC):
                cum.append(cum[-1] + pr[c])
            tails.append(cum[-1])
            queue.append(pltpu.bitcast(jnp.concatenate(cum, axis=0), U32))

        def pending():
            return bool(groups or queue)

        def pace(lhs, skip=0):
            if not pending():
                return lhs
            lb = pltpu.bitcast(lhs, U32)
            r0 = r1 = skip * 8
            got = []
            while r1 < lb.shape[0] and pending():
                if not queue:
                    tail_group()
                a = queue.pop(0)
                n = min(a.shape[0], lb.shape[0] - r1)
                if n < a.shape[0]:
                    queue.append(a[n:])
                    a = a[:n]
                got.append(a)
                r1 += n
            mid = jnp.where(always, lb[r0:r1, :256], jnp.concatenate(got, axis=0) if len(got) > 1 else got[0])
            if lb.shape[1] > 256:
                mid = jnp.concatenate([mid, lb[r0:r1, 256:]], axis=1)
            parts = ([lb[:r0]] if r0 else []) + [mid] + ([lb[r1:]] if r1 < lb.shape[0] else [])
            return pltpu.bitcast(jnp.concatenate(parts, axis=0) if len(parts) > 1 else mid, BF16)

        def q_rest(n):
            x = pace(x_s[jp, R:], (1, 12, 0, 0)[n])
            w = wq_s[j & 15, :, n * 128:(n + 1) * 128]
            q = (jnp.dot(x, w, preferred_element_type=F32) * SCALE).astype(BF16)
            store_q(j, q, R, n * 128)

        def q_head():
            assert not pending()
            main = jnp.dot(x_s[jp, :R, :DM], wq_s[j & 15, :DM, :], preferred_element_type=F32)
            t = jnp.stack(tails)
            tail = jnp.concatenate(
                [jnp.concatenate([t[:, n * 8:(n + 1) * 8, hf * 128:(hf + 1) * 128] for n in range(4)], axis=2)
                 for hf in range(2)], axis=1).reshape(R, W)
            store_q(j, ((main + tail) * SCALE).astype(BF16), 0, 0)

        def qk(b):
            q = q_s[i & 7, b]
            if pending():
                s = jnp.concatenate(
                    [lax.dot_general(pace(q), k_s[slot, b, r * 256:(r + 1) * 256, :], NT,
                                     preferred_element_type=F32) for r in range(4)], axis=1)
            else:
                s = lax.dot_general(q, k_s[slot, b], NT, preferred_element_type=F32)
            m = jnp.max(s, axis=-1, keepdims=True)
            pb = jnp.exp2(s - m).astype(BF16)
            pf = pb.astype(F32)
            lp = pf[:, 0:128]
            for c in range(1, SK // 128):
                lp = lp + pf[:, c * 128:(c + 1) * 128]
            return pb, lp

        def pv(b, pb, lp):
            o = jnp.dot(pb, v_s[slot, b], preferred_element_type=F32)
            lp = jnp.where(always, lp, o[:, 0:128])
            if staged:
                zt = staged.pop()
                ls = [lp[:128], lp[128:256], lp[256:]]
                for c in range(4):
                    ls[c % 2] = jnp.where(always, ls[c % 2], zt[:, c * 128:(c + 1) * 128])
                lp = jnp.concatenate(ls, axis=0)
            l = jnp.sum(lp, axis=-1, keepdims=True)
            r = pl.reciprocal(l, approx=True)
            r = r * (2.0 - l * r)
            o = (o * r).astype(BF16)
            o_s[b * SQ:(b + 1) * SQ, :DH] = o[:SQ]
            o_s[b * SQ:(b + 1) * SQ, DH:] = o[SQ:]

        def oproj(n):
            cs = slice(n * 128, (n + 1) * 128)
            part = lax.dot_general(pace(wo_s[i & 15]), o_s[cs, :], NT, preferred_element_type=F32)
            if not final:
                if n >= 6:
                    deps.append(part)
                acc_s[ab, :, cs] = jnp.where(h == 0, 0.0, acc_s[ab, :, cs]) + part
            else:
                fin = acc_s[ab, :, cs] + part
                acc_s[ab, :, cs] = fin
                r = fin[:DR]
                ra = jnp.where(ab == 0, r, mid_s[:, cs])
                mid_s[:, cs] = ra
                zt = jnp.concatenate([fin[DR:], ra, r], axis=0).T
                st_s[p, cs, :] = zt.astype(BF16)
                staged.append(zt)

        def write_back(n):
            r = pl.multiple_of((p >> 1) * T + n * 128, 128)
            c = pl.multiple_of(ab * W, W)

            @pl.when(h == HKV - 1)
            def _():
                copy(st_s.at[p, pl.ds(n * 128, 128), pl.ds(0, DM)],
                     out.at[pl.ds(r, 128), pl.ds(c, DM)], out_sem.at[0]).start()

            @pl.when(jnp.logical_and(h == HKV - 1, ab == 1))
            def _():
                copy(st_s.at[p, pl.ds(n * 128, 128), pl.ds(DM, 128)],
                     out.at[pl.ds(r, 128), pl.ds(DM, 128)], out_sem.at[1]).start()

        def prefetch_q_operands(jn):
            n = jnp.minimum(jn, NBLK - 1)
            start_from(jn < 16, (n >> 3) & 1, lambda a: (wq_copy(a, n),))
            start_from(jnp.logical_and(jn < NBLK, (n & 7) == 0), (n >> 3) & 1,
                       lambda a: (x_copy(a, n >> 3),))
            start_from(jn + 1 < LOOK + 16, ((jn + 1) >> 3) & 1, lambda a: (wt_copy(a, jn + 1),))

        live = {}
        for tok in (Y_ORDER if final else X_ORDER).split():
            kind, n = tok[0], int(tok[1:])
            if kind == "k":
                live[n] = qk(n)
            elif kind == "v":
                pv(n, *live.pop(n))
            elif kind == "o":
                oproj(n)
            elif kind == "r":
                q_rest(n)
            elif kind == "z":
                q_head()
            elif kind == "t":
                write_back(n)
            elif kind == "w":
                build_wb(j + 1, always, jnp.concatenate(deps, axis=0))
            elif kind == "b":
                build_xb(jnp.minimum(p + 2, 3), p & 1, 0, NG)
            else:
                prefetch_q_operands(j + 2)

    def fence():
        pl.semaphore_signal(bar_sem, 1)
        pl.semaphore_wait(bar_sem, 1)

    half = T // 2
    xh = [copy(xa.at[pl.ds(c * half, half)], x_s.at[0, pl.ds(c * half, half)], x_sem.at[c])
          for c in range(2)]
    wh = [copy(wqa.at[:, pl.ds(c * DH, DH)], wq_s.at[0, :, pl.ds(c * DH, DH)], wq_sem.at[7 * c])
          for c in range(2)]
    for c in range(2):
        xh[c].start()
        wh[c].start()
        fence()
    for c in ([xt_copy(0), xt_copy(1), wt_copy(0, LOOK), wt_copy(0, LOOK + 1)]
              + [wq_copy(0, j) for j in range(1, LOOK)]):
        c.start()
    fence()
    for c in kv_copies(0, 0) + wo_copies(0, 0) + (wq_copy(0, LOOK),):
        c.start()
    fence()
    for c in (wq_copy(0, LOOK + 1), wt_copy(0, LOOK + 2), xt_copy(2), xt_copy(3)):
        c.start()

    def qproj0(rh, ch):
        x = x_s[0, rh * half:(rh + 1) * half]
        w = wq_s[0, :, ch * DH:(ch + 1) * DH]
        q = (jnp.dot(x, w, preferred_element_type=F32) * SCALE).astype(BF16)
        store_q(0, q, rh * half, ch * DH)

    xh[0].wait()
    wh[0].wait()
    qproj0(0, 0)
    xh[1].wait()
    wh[1].wait()
    qproj0(0, 1)
    qproj0(1, 0)
    qproj0(1, 1)
    xt_copy(0).wait()
    xt_copy(1).wait()
    wt_copy(0, LOOK).wait()

    ngp = (NG + 1) // 2

    def qproj_ahead(jj, carry):
        j = 1 + jj
        wq_copy(0, j).wait()
        build_xb(jj >> 1, jj >> 1, (jj & 1) * (NG - ngp), ngp)
        qs = []
        for n in range(4):
            qf = jnp.dot(x_s[0], wq_s[j, :, n * 128:(n + 1) * 128], preferred_element_type=F32)
            qs.append(qf)
            store_q(j, (qf * SCALE).astype(BF16), 0, n * 128)
        build_wb(LOOK, jj >= 0, jnp.concatenate(qs[:2], axis=0))
        return carry
    lax.fori_loop(0, LOOK - 1, qproj_ahead, 0)

    def phase(p, carry):
        nx = jnp.where(p == 3, HKV - (LOOK - 3), HKV - 1)

        def x_body(h, c):
            block(p * HKV + h, False)
            return c
        lax.fori_loop(0, nx, x_body, 0)

        def y_body(h, c):
            block(p * HKV + h, True)
            return c
        lax.fori_loop(nx, HKV, y_body, 0)
        return carry
    lax.fori_loop(0, 4, phase, 0)

    wait_for(st_s.at[:, :, pl.ds(0, DM)], out_sem.at[0])
    wait_for(st_s.at[pl.ds(0, 2), :, pl.ds(DM, 128)], out_sem.at[1])


@jax.jit
def pallas_concat_heads__gqa_block_cached__gqa_block_cached__near_ridge_kernel(
    A_x: jax.Array,
    A_k_cache: jax.Array,
    A_v_cache: jax.Array,
    A_wq: jax.Array,
    A_wo: jax.Array,
    B_x: jax.Array,
    B_k_cache: jax.Array,
    B_v_cache: jax.Array,
    B_wq: jax.Array,
    B_wo: jax.Array,
):
    assert A_x.shape == (B, SQ, D) and A_k_cache.shape == (B, HKV, SK, DH)
    any_spec = pl.BlockSpec(memory_space=pl.ANY)
    out = pl.pallas_call(
        _kernel,
        in_specs=[any_spec] * 10,
        out_specs=any_spec,
        out_shape=jax.ShapeDtypeStruct((B * SQ, 2 * D), BF16),
        scratch_shapes=[
            pltpu.VMEM((4, T, D), BF16),
            pltpu.VMEM((16, D, W), BF16),
            pltpu.VMEM((16, D, W), BF16),
            pltpu.VMEM((2, NB, SK, DH), BF16),
            pltpu.VMEM((2, NB, SK, DH), BF16),
            pltpu.VMEM((8, NB, 2 * SQ, DH), BF16),
            pltpu.VMEM((T, W), BF16),
            pltpu.VMEM((2, D, T), F32),
            pltpu.VMEM((DR, T), F32),
            pltpu.VMEM((4, T, W), BF16),
            pltpu.VMEM((4, R, DR), BF16),
            pltpu.VMEM((2, NG, DR, 8, 256), F32),
            pltpu.VMEM((NC, 4, KC, 8, 128), F32),
            pltpu.VMEM((16, DR, W), BF16),
            pltpu.SemaphoreType.DMA((2, 2)),
            pltpu.SemaphoreType.DMA((8,)),
            pltpu.SemaphoreType.DMA((2,)),
            pltpu.SemaphoreType.DMA((4,)),
            pltpu.SemaphoreType.DMA((2,)),
            pltpu.SemaphoreType.DMA((3,)),
            pltpu.SemaphoreType.DMA((4,)),
            pltpu.SemaphoreType.REGULAR,
        ],
        compiler_params=pltpu.CompilerParams(
            disable_bounds_checks=True,
            vmem_limit_bytes=112 * 1024 * 1024),
    )(A_x.reshape(B * SQ, D), A_k_cache, A_v_cache, A_wq, A_wo.T,
      B_x.reshape(B * SQ, D), B_k_cache, B_v_cache, B_wq, B_wo.T)
    return out.reshape(B, SQ, 2 * D)
```

```python
import jax
import jax.numpy as jnp
from jax import lax
import jax.experimental.pallas as pl
import jax.experimental.pallas.tpu as pltpu

LOG2E = 1.4426950408889634
NT = (((1,), (1,)), ((), ()))

B, SQ, D = 16, 144, 448
HKV, SK, DH = 8, 1024, 256
NB = 8
T = NB * SQ
W = 2 * DH
DM = 384
DR = D - DM
LOOK = 5
NBLK = 32
NG = 30
R = NG * 16
KC = 8
NC = DR // KC

X_ORDER = ("r0 k0 k1 v0 k2 v1 o0 k3 v2 o1 k4 v3 o2 k5 v4 o3 k6 v5 o4 k7 r1 v6 o5 "
           "r2 v7 z0 o6 o7 o8 w0 r3 n0")
Y_ORDER = ("k0 k1 v0 k2 v1 o0 t0 k3 v2 o1 t1 k4 v3 o2 t2 k5 v4 o3 t3 k6 v5 o4 "
           "t4 k7 v6 o5 t5 v7 o6 t6 o7 t7 o8 t8 b0")

F32 = jnp.float32
BF16 = jnp.bfloat16
U32 = jnp.uint32
SCALE = (DH ** -0.5) * LOG2E


def _kernel(xa, ka, va, wqa, wota, xb, kb, vb, wqb, wotb, out,
            x_s, wq_s, wo_s, k_s, v_s, q_s, o_s, acc_s, mid_s, st_s, xt_s, xb_s, wb_s, wt_s,
            kv_sem, wq_sem, wo_sem, x_sem, out_sem, xt_sem, wt_sem, bar_sem):
    srcs = ((xa, ka, va, wqa, wota), (xb, kb, vb, wqb, wotb))
    copy = pltpu.make_async_copy

    def wait_for(dst, sem):
        copy(dst, dst, sem).wait()

    def kv_copies(ab, i):
        g, h, slot = i >> 4, i & 7, i & 1
        return (copy(srcs[ab][1].at[pl.ds(g * NB, NB), h], k_s.at[slot], kv_sem.at[0, slot]),
                copy(srcs[ab][2].at[pl.ds(g * NB, NB), h], v_s.at[slot], kv_sem.at[1, slot]))

    def wq_copy(ab, j):
        c = pl.multiple_of((j & 7) * W, W)
        return copy(srcs[ab][3].at[:, pl.ds(c, W)], wq_s.at[j & 15], wq_sem.at[j & 7])

    def wt_copy(ab, j):
        c = pl.multiple_of((j & 7) * W, W)
        return copy(srcs[ab][3].at[pl.ds(DM, DR), pl.ds(c, W)], wt_s.at[j & 15], wt_sem.at[j & 3])

    def wo_copies(ab, i):
        c = pl.multiple_of((i & 7) * W, W)
        wot, dst, sem = srcs[ab][4], wo_s.at[i & 15], wo_sem.at[i & 1]
        if ab == 1:
            return (copy(wot.at[:, pl.ds(c, W)], dst, sem),)
        return (copy(wot.at[pl.ds(DM, DR), pl.ds(c, W)], dst.at[pl.ds(0, DR)], sem),
                copy(wot.at[pl.ds(0, DM), pl.ds(c, W)], dst.at[pl.ds(DR, DM)], sem))

    def x_copy(ab, p):
        r = pl.multiple_of((p >> 1) * T, T)
        return copy(srcs[ab][0].at[pl.ds(r, T)], x_s.at[p], x_sem.at[p])

    def xt_copy(p):
        return copy(srcs[p & 1][0].at[pl.ds((p >> 1) * T, R), pl.ds(DM, DR)],
                    xt_s.at[pl.ds(p * R, R)], xt_sem.at[p])

    def start_from(cond, ab_dyn, fn):
        for ab in range(2):
            @pl.when(jnp.logical_and(cond, ab_dyn == ab))
            def _():
                for c in fn(ab):
                    c.start()

    def store_q(j, q, row0, col0):
        nrow, ncol = q.shape
        cw = min(ncol, DH)
        for c0 in range(col0, col0 + ncol, cw):
            head, cc = c0 // DH, c0 % DH
            r = row0
            while r < row0 + nrow:
                b, off = r // SQ, r % SQ
                n = min(SQ - off, row0 + nrow - r)
                q_s[j & 7, b, head * SQ + off:head * SQ + off + n, cc:cc + cw] = (
                    q[r - row0:r - row0 + n, c0 - col0:c0 - col0 + cw])
                r += n

    def halves_on_lanes(v):
        v = v.reshape(v.shape[0] // 16, 16, 128)
        return jnp.concatenate([v[:, :8], v[:, 8:]], axis=2)

    def build_xb(gs, gd, ng):
        xt = pltpu.bitcast(xt_s[pl.ds(pl.multiple_of(gs * 16, 16), ng * 16), :], U32)
        for k in range(DR):
            bc = jnp.broadcast_to(xt[:, k:k + 1], (ng * 8, 128))
            xb_s[pl.ds(gd, ng), k] = halves_on_lanes(pltpu.bitcast(bc, BF16).astype(F32))

    def build_wb(j, always, dep):
        w32 = wt_s[j & 15].astype(F32)
        step = dep.shape[0] // 256 * 8
        for c in range(4):
            dc = jnp.concatenate([dep[(c * 8 + r) * step:(c * 8 + r) * step + 8] for r in range(8)], axis=0)
            wc = jnp.where(always, w32[:, c * 128:(c + 1) * 128], dc)
            wb_s[:, c] = jnp.broadcast_to(wc[:, None, :], (DR, 8, 128)).reshape(NC, KC, 8, 128)

    def block(i, final):
        slot, p, h = i & 1, i >> 3, i & 7
        ab = p & 1
        j = i + LOOK - p
        jp = j >> 3

        wait_for(k_s.at[slot], kv_sem.at[0, slot])
        wait_for(v_s.at[slot], kv_sem.at[1, slot])

        @pl.when(i < 16)
        def _():
            wait_for(wo_s.at[i & 15], wo_sem.at[i & 1])
        if not final:
            @pl.when(j < 16)
            def _():
                wait_for(wq_s.at[j & 15], wq_sem.at[j & 7])

            @pl.when((j & 7) == 0)
            def _():
                wait_for(x_s.at[jp], x_sem.at[jp])

            @pl.when(j + 1 < LOOK + 16)
            def _():
                wait_for(wt_s.at[(j + 1) & 15], wt_sem.at[(j + 1) & 3])
        else:
            @pl.when(p == 0)
            def _():
                xt_copy(3).wait()

        nxt = jnp.minimum(i + 1, NBLK - 1)
        start_from(i < NBLK - 1, (nxt >> 3) & 1, lambda a: kv_copies(a, nxt))
        start_from(i < 15, (nxt >> 3) & 1, lambda a: wo_copies(a, nxt))

        always = i >= 0
        staged = []

        groups = [] if final else list(range(NG))
        tails, queue, deps = [], [], []

        def tail_group():
            g = groups.pop(0)
            x = xb_s[jnp.where(jp == 3, 0, jp) * NG + g].reshape(NC, 1, KC, 8, 256)
            w = wb_s[...]
            pr = jnp.sum(x * jnp.concatenate([w, w], axis=4), axis=2).reshape(NC, 32, 256)
            cum = [pr[0]]
            for c in range(1, NC):
                cum.append(cum[-1] + pr[c])
            tails.append(cum[-1])
            queue.append(pltpu.bitcast(jnp.concatenate(cum, axis=0), U32))

        def pending():
            return bool(groups or queue)

        def pace(lhs, skip=0, cut=0):
            if not pending():
                return lhs
            lb = pltpu.bitcast(lhs, U32)
            r0 = r1 = skip * 8
            lim = lb.shape[0] - cut * 8
            got = []
            while r1 < lim and pending():
                if not queue:
                    tail_group()
                a = queue.pop(0)
                n = min(a.shape[0], lim - r1)
                if n < a.shape[0]:
                    queue.append(a[n:])
                    a = a[:n]
                got.append(a)
                r1 += n
            mid = jnp.where(always, lb[r0:r1, :256], jnp.concatenate(got, axis=0) if len(got) > 1 else got[0])
            if lb.shape[1] > 256:
                mid = jnp.concatenate([mid, lb[r0:r1, 256:]], axis=1)
            parts = ([lb[:r0]] if r0 else []) + [mid] + ([lb[r1:]] if r1 < lb.shape[0] else [])
            return pltpu.bitcast(jnp.concatenate(parts, axis=0) if len(parts) > 1 else mid, BF16)

        def q_rest(n):
            x = pace(x_s[jp, R:], (1, 12, 0, 0)[n])
            w = wq_s[j & 15, :, n * 128:(n + 1) * 128]
            q = (jnp.dot(x, w, preferred_element_type=F32) * SCALE).astype(BF16)
            store_q(j, q, R, n * 128)

        def q_head():
            assert not pending()
            main = jnp.dot(x_s[jp, :R, :DM], wq_s[j & 15, :DM, :], preferred_element_type=F32)
            t = jnp.stack(tails)
            tail = jnp.concatenate(
                [jnp.concatenate([t[:, n * 8:(n + 1) * 8, hf * 128:(hf + 1) * 128] for n in range(4)], axis=2)
                 for hf in range(2)], axis=1).reshape(R, W)
            store_q(j, ((main + tail) * SCALE).astype(BF16), 0, 0)

        def qk(b):
            q = q_s[i & 7, b]
            if pending():
                s = jnp.concatenate(
                    [lax.dot_general(pace(q, 0, 2 if r == 3 else 0), k_s[slot, b, r * 256:(r + 1) * 256, :], NT,
                                     preferred_element_type=F32) for r in range(4)], axis=1)
            else:
                s = lax.dot_general(q, k_s[slot, b], NT, preferred_element_type=F32)
            m = jnp.max(s, axis=-1, keepdims=True)
            pf = jnp.exp2(s - m)
            u = pltpu.bitcast(pf.astype(BF16), U32)
            lp, parts = None, []
            for hf in range(2):
                for c in range(4 * hf, 4 * hf + 4):
                    t = pf[:, c * 128:(c + 1) * 128]
                    lp = t if lp is None else lp + t
                a = halves_on_lanes(pltpu.bitcast(lp, U32)).reshape(SQ, 256)
                parts += [jnp.where(always, u[:, hf * 512:hf * 512 + 256], a),
                          u[:, hf * 512 + 256:hf * 512 + 512]]
            return pltpu.bitcast(jnp.concatenate(parts, axis=1), BF16), lp

        def pv(b, pb, lp):
            if pending():
                o = jnp.concatenate(
                    [jnp.dot(pb, v_s[slot, b, :, :128], preferred_element_type=F32),
                     jnp.dot(jnp.concatenate([pb[:, :512], pace(pb[:, 512:])], axis=1),
                             v_s[slot, b, :, 128:], preferred_element_type=F32)], axis=1)
            else:
                o = jnp.dot(pb, v_s[slot, b], preferred_element_type=F32)
            lp = jnp.where(always, lp, o[:, 0:128])
            if staged:
                zt = staged.pop()
                ls = [lp[:128], lp[128:256], lp[256:]]
                for c in range(4):
                    ls[c % 2] = jnp.where(always, ls[c % 2], zt[:, c * 128:(c + 1) * 128])
                lp = jnp.concatenate(ls, axis=0)
            l = jnp.sum(lp, axis=-1, keepdims=True)
            r = pl.reciprocal(l, approx=True)
            r = r * (2.0 - l * r)
            o = (o * r).astype(BF16)
            o_s[b * SQ:(b + 1) * SQ, :DH] = o[:SQ]
            o_s[b * SQ:(b + 1) * SQ, DH:] = o[SQ:]

        def oproj(n):
            cs = slice(n * 128, (n + 1) * 128)
            part = lax.dot_general(pace(wo_s[i & 15]), o_s[cs, :], NT, preferred_element_type=F32)
            if not final:
                if n >= 6:
                    deps.append(part)
                acc_s[ab, :, cs] = jnp.where(h == 0, 0.0, acc_s[ab, :, cs]) + part
            else:
                fin = acc_s[ab, :, cs] + part
                acc_s[ab, :, cs] = fin
                r = fin[:DR]
                ra = jnp.where(ab == 0, r, mid_s[:, cs])
                mid_s[:, cs] = ra
                zt = jnp.concatenate([fin[DR:], ra, r], axis=0).T
                st_s[p, cs, :] = zt.astype(BF16)
                staged.append(zt)

        def write_back(n):
            r = pl.multiple_of((p >> 1) * T + n * 128, 128)
            c = pl.multiple_of(ab * W, W)

            @pl.when(h == HKV - 1)
            def _():
                copy(st_s.at[p, pl.ds(n * 128, 128), pl.ds(0, DM)],
                     out.at[pl.ds(r, 128), pl.ds(c, DM)], out_sem.at[0]).start()

            @pl.when(jnp.logical_and(h == HKV - 1, ab == 1))
            def _():
                copy(st_s.at[p, pl.ds(n * 128, 128), pl.ds(DM, 128)],
                     out.at[pl.ds(r, 128), pl.ds(DM, 128)], out_sem.at[1]).start()

        def prefetch_q_operands(jn):
            n = jnp.minimum(jn, NBLK - 1)
            start_from(jn < 16, (n >> 3) & 1, lambda a: (wq_copy(a, n),))
            start_from(jnp.logical_and(jn < NBLK, (n & 7) == 0), (n >> 3) & 1,
                       lambda a: (x_copy(a, n >> 3),))
            start_from(jn + 1 < LOOK + 16, ((jn + 1) >> 3) & 1, lambda a: (wt_copy(a, jn + 1),))

        live = {}
        for tok in (Y_ORDER if final else X_ORDER).split():
            kind, n = tok[0], int(tok[1:])
            if kind == "k":
                live[n] = qk(n)
            elif kind == "v":
                pv(n, *live.pop(n))
            elif kind == "o":
                oproj(n)
            elif kind == "r":
                q_rest(n)
            elif kind == "z":
                q_head()
            elif kind == "t":
                write_back(n)
            elif kind == "w":
                build_wb(j + 1, always, jnp.concatenate(deps, axis=0))
            elif kind == "b":
                g0 = (p & 1) * (NG // 2)
                build_xb(3 * NG + g0, g0, NG // 2)
            else:
                prefetch_q_operands(j + 2)

    def fence():
        pl.semaphore_signal(bar_sem, 1)
        pl.semaphore_wait(bar_sem, 1)

    half = T // 2
    xh = [copy(xa.at[pl.ds(c * half, half)], x_s.at[0, pl.ds(c * half, half)], x_sem.at[c])
          for c in range(2)]
    wh = [copy(wqa.at[:, pl.ds(c * DH, DH)], wq_s.at[0, :, pl.ds(c * DH, DH)], wq_sem.at[7 * c])
          for c in range(2)]
    for c in range(2):
        xh[c].start()
        wh[c].start()
        fence()
    for c in ([xt_copy(0), xt_copy(1), xt_copy(2), wt_copy(0, LOOK), wt_copy(0, LOOK + 1)]
              + [wq_copy(0, j) for j in range(1, LOOK)]):
        c.start()
    fence()
    for c in kv_copies(0, 0) + wo_copies(0, 0) + (wq_copy(0, LOOK),):
        c.start()
    fence()
    for c in (wq_copy(0, LOOK + 1), wt_copy(0, LOOK + 2), xt_copy(3)):
        c.start()

    def qproj0(rh, ch):
        x = x_s[0, rh * half:(rh + 1) * half]
        w = wq_s[0, :, ch * DH:(ch + 1) * DH]
        q = (jnp.dot(x, w, preferred_element_type=F32) * SCALE).astype(BF16)
        store_q(0, q, rh * half, ch * DH)

    xh[0].wait()
    wh[0].wait()
    qproj0(0, 0)
    xh[1].wait()
    wh[1].wait()
    qproj0(0, 1)
    qproj0(1, 0)
    qproj0(1, 1)
    for c in range(3):
        xt_copy(c).wait()
    wt_copy(0, LOOK).wait()

    ngp = -(-3 * NG // (LOOK - 1))

    def qproj_ahead(jj, carry):
        j = 1 + jj
        wq_copy(0, j).wait()
        g0 = jnp.minimum(jj * ngp, 3 * NG - ngp)
        build_xb(g0, g0, ngp)
        qs = []
        for n in range(4):
            qf = jnp.dot(x_s[0], wq_s[j, :, n * 128:(n + 1) * 128], preferred_element_type=F32)
            qs.append(qf)
            store_q(j, (qf * SCALE).astype(BF16), 0, n * 128)
        build_wb(LOOK, jj >= 0, jnp.concatenate(qs[:2], axis=0))
        return carry
    lax.fori_loop(0, LOOK - 1, qproj_ahead, 0)

    def phase(p, carry):
        nx = jnp.where(p == 3, HKV - (LOOK - 3), HKV - 1)

        def x_body(h, c):
            block(p * HKV + h, False)
            return c
        lax.fori_loop(0, nx, x_body, 0)

        def y_body(h, c):
            block(p * HKV + h, True)
            return c
        lax.fori_loop(nx, HKV, y_body, 0)
        return carry
    lax.fori_loop(0, 4, phase, 0)

    wait_for(st_s.at[:, :, pl.ds(0, DM)], out_sem.at[0])
    wait_for(st_s.at[pl.ds(0, 2), :, pl.ds(DM, 128)], out_sem.at[1])


@jax.jit
def pallas_concat_heads__gqa_block_cached__gqa_block_cached__near_ridge_kernel(
    A_x: jax.Array,
    A_k_cache: jax.Array,
    A_v_cache: jax.Array,
    A_wq: jax.Array,
    A_wo: jax.Array,
    B_x: jax.Array,
    B_k_cache: jax.Array,
    B_v_cache: jax.Array,
    B_wq: jax.Array,
    B_wo: jax.Array,
):
    assert A_x.shape == (B, SQ, D) and A_k_cache.shape == (B, HKV, SK, DH)
    any_spec = pl.BlockSpec(memory_space=pl.ANY)
    out = pl.pallas_call(
        _kernel,
        in_specs=[any_spec] * 10,
        out_specs=any_spec,
        out_shape=jax.ShapeDtypeStruct((B * SQ, 2 * D), BF16),
        scratch_shapes=[
            pltpu.VMEM((4, T, D), BF16),
            pltpu.VMEM((16, D, W), BF16),
            pltpu.VMEM((16, D, W), BF16),
            pltpu.VMEM((2, NB, SK, DH), BF16),
            pltpu.VMEM((2, NB, SK, DH), BF16),
            pltpu.VMEM((8, NB, 2 * SQ, DH), BF16),
            pltpu.VMEM((T, W), BF16),
            pltpu.VMEM((2, D, T), F32),
            pltpu.VMEM((DR, T), F32),
            pltpu.VMEM((4, T, W), BF16),
            pltpu.VMEM((4 * R, DR), BF16),
            pltpu.VMEM((3 * NG, DR, 8, 256), F32),
            pltpu.VMEM((NC, 4, KC, 8, 128), F32),
            pltpu.VMEM((16, DR, W), BF16),
            pltpu.SemaphoreType.DMA((2, 2)),
            pltpu.SemaphoreType.DMA((8,)),
            pltpu.SemaphoreType.DMA((2,)),
            pltpu.SemaphoreType.DMA((4,)),
            pltpu.SemaphoreType.DMA((2,)),
            pltpu.SemaphoreType.DMA((4,)),
            pltpu.SemaphoreType.DMA((4,)),
            pltpu.SemaphoreType.REGULAR,
        ],
        compiler_params=pltpu.CompilerParams(
            disable_bounds_checks=True,
            vmem_limit_bytes=120 * 1024 * 1024),
    )(A_x.reshape(B * SQ, D), A_k_cache, A_v_cache, A_wq, A_wo.T,
      B_x.reshape(B * SQ, D), B_k_cache, B_v_cache, B_wq, B_wo.T)
    return out.reshape(B, SQ, 2 * D)
```

```python
import jax
import jax.numpy as jnp
from jax import lax
import jax.experimental.pallas as pl
import jax.experimental.pallas.tpu as pltpu

LOG2E = 1.4426950408889634
NT = (((1,), (1,)), ((), ()))

B, SQ, D = 16, 144, 448
HKV, SK, DH = 8, 1024, 256
NB = 8
T = NB * SQ
W = 2 * DH
DM = 384
DR = D - DM
LOOK = 5
NBLK = 32
NG = 30
R = NG * 16
KC = 8
NC = DR // KC

X_ORDER = ("r0 k0 k1 v0 k2 v1 o0 k3 v2 o1 k4 v3 o2 k5 v4 o3 k6 v5 o4 k7 r1 v6 o5 "
           "r2 v7 z0 o6 o7 o8 w0 r3 n0")
Y_ORDER = ("k0 k1 v0 k2 v1 o0 t0 k3 v2 o1 t1 k4 v3 o2 t2 k5 v4 o3 t3 k6 v5 o4 "
           "t4 k7 v6 o5 t5 v7 o6 t6 o7 t7 o8 t8 b0")

F32 = jnp.float32
BF16 = jnp.bfloat16
U32 = jnp.uint32
SCALE = (DH ** -0.5) * LOG2E


def _kernel(xa, ka, va, wqa, wota, xb, kb, vb, wqb, wotb, out,
            x_s, wq_s, wo_s, k_s, v_s, q_s, o_s, acc_s, mid_s, st_s, xt_s, xb_s, wb_s, wt_s,
            kv_sem, wq_sem, wo_sem, x_sem, out_sem, xt_sem, wt_sem, bar_sem):
    srcs = ((xa, ka, va, wqa, wota), (xb, kb, vb, wqb, wotb))
    copy = pltpu.make_async_copy

    def wait_for(dst, sem):
        copy(dst, dst, sem).wait()

    def kv_copies(ab, i):
        g, h, slot = i >> 4, i & 7, i & 1
        return (copy(srcs[ab][1].at[pl.ds(g * NB, NB), h], k_s.at[slot], kv_sem.at[0, slot]),
                copy(srcs[ab][2].at[pl.ds(g * NB, NB), h], v_s.at[slot], kv_sem.at[1, slot]))

    def wq_copy(ab, j):
        c = pl.multiple_of((j & 7) * W, W)
        return copy(srcs[ab][3].at[:, pl.ds(c, W)], wq_s.at[j & 15], wq_sem.at[j & 7])

    def wt_copy(ab, j):
        c = pl.multiple_of((j & 7) * W, W)
        return copy(srcs[ab][3].at[pl.ds(DM, DR), pl.ds(c, W)], wt_s.at[j & 15], wt_sem.at[j & 3])

    def wo_copies(ab, i):
        c = pl.multiple_of((i & 7) * W, W)
        wot, dst, sem = srcs[ab][4], wo_s.at[i & 15], wo_sem.at[i & 1]
        if ab == 1:
            return (copy(wot.at[:, pl.ds(c, W)], dst, sem),)
        return (copy(wot.at[pl.ds(DM, DR), pl.ds(c, W)], dst.at[pl.ds(0, DR)], sem),
                copy(wot.at[pl.ds(0, DM), pl.ds(c, W)], dst.at[pl.ds(DR, DM)], sem))

    def x_copy(ab, p):
        r = pl.multiple_of((p >> 1) * T, T)
        return copy(srcs[ab][0].at[pl.ds(r, T)], x_s.at[p], x_sem.at[p])

    def xt_copy(p):
        return copy(srcs[p & 1][0].at[pl.ds((p >> 1) * T, R), pl.ds(DM, DR)],
                    xt_s.at[pl.ds(p * R, R)], xt_sem.at[p])

    def start_from(cond, ab_dyn, fn):
        for ab in range(2):
            @pl.when(jnp.logical_and(cond, ab_dyn == ab))
            def _():
                for c in fn(ab):
                    c.start()

    def store_q(j, q, row0, col0):
        nrow, ncol = q.shape
        cw = min(ncol, DH)
        for c0 in range(col0, col0 + ncol, cw):
            head, cc = c0 // DH, c0 % DH
            r = row0
            while r < row0 + nrow:
                b, off = r // SQ, r % SQ
                n = min(SQ - off, row0 + nrow - r)
                q_s[j & 7, b, head * SQ + off:head * SQ + off + n, cc:cc + cw] = (
                    q[r - row0:r - row0 + n, c0 - col0:c0 - col0 + cw])
                r += n

    def halves_on_lanes(v):
        v = v.reshape(v.shape[0] // 16, 16, 128)
        return jnp.concatenate([v[:, :8], v[:, 8:]], axis=2)

    def build_xb(gs, gd, ng):
        xt = pltpu.bitcast(xt_s[pl.ds(pl.multiple_of(gs * 16, 16), ng * 16), :], U32)
        for k in range(DR):
            bc = jnp.broadcast_to(xt[:, k:k + 1], (ng * 8, 128))
            xb_s[pl.ds(gd, ng), k] = halves_on_lanes(pltpu.bitcast(bc, BF16).astype(F32))

    def build_wb(j, always, dep):
        w32 = wt_s[j & 15].astype(F32)
        step = dep.shape[0] // 256 * 8
        for c in range(4):
            dc = jnp.concatenate([dep[(c * 8 + r) * step:(c * 8 + r) * step + 8] for r in range(8)], axis=0)
            wc = jnp.where(always, w32[:, c * 128:(c + 1) * 128], dc)
            wb_s[:, c] = jnp.broadcast_to(wc[:, None, :], (DR, 8, 128)).reshape(NC, KC, 8, 128)

    def block(i, final):
        slot, p, h = i & 1, i >> 3, i & 7
        ab = p & 1
        j = i + LOOK - p
        jp = j >> 3

        wait_for(k_s.at[slot], kv_sem.at[0, slot])
        wait_for(v_s.at[slot], kv_sem.at[1, slot])

        @pl.when(i < 16)
        def _():
            wait_for(wo_s.at[i & 15], wo_sem.at[i & 1])
        if not final:
            @pl.when(j < 16)
            def _():
                wait_for(wq_s.at[j & 15], wq_sem.at[j & 7])

            @pl.when((j & 7) == 0)
            def _():
                wait_for(x_s.at[jp], x_sem.at[jp])

            @pl.when(j + 1 < LOOK + 16)
            def _():
                wait_for(wt_s.at[(j + 1) & 15], wt_sem.at[(j + 1) & 3])
        else:
            @pl.when(p == 0)
            def _():
                xt_copy(3).wait()

        nxt = jnp.minimum(i + 1, NBLK - 1)
        start_from(i < NBLK - 1, (nxt >> 3) & 1, lambda a: kv_copies(a, nxt))
        start_from(i < 15, (nxt >> 3) & 1, lambda a: wo_copies(a, nxt))

        always = i >= 0
        staged = []

        groups = [] if final else list(range(NG))
        tails, queue, deps = [], [], []

        def tail_group():
            g = groups.pop(0)
            x = xb_s[jnp.where(jp == 3, 0, jp) * NG + g].reshape(NC, 1, KC, 8, 256)
            w = wb_s[...]
            pr = jnp.sum(x * jnp.concatenate([w, w], axis=4), axis=2).reshape(NC, 32, 256)
            cum = [pr[0]]
            for c in range(1, NC):
                cum.append(cum[-1] + pr[c])
            tails.append(cum[-1])
            queue.append(pltpu.bitcast(jnp.concatenate(cum, axis=0), U32))

        def pending():
            return bool(groups or queue)

        def pace(lhs, skip=0, cut=0):
            if not pending():
                return lhs
            lb = pltpu.bitcast(lhs, U32)
            r0 = r1 = skip * 8
            lim = lb.shape[0] - cut * 8
            got = []
            while r1 < lim and pending():
                if not queue:
                    tail_group()
                a = queue.pop(0)
                n = min(a.shape[0], lim - r1)
                if n < a.shape[0]:
                    queue.append(a[n:])
                    a = a[:n]
                got.append(a)
                r1 += n
            mid = jnp.where(always, lb[r0:r1, :256], jnp.concatenate(got, axis=0) if len(got) > 1 else got[0])
            if lb.shape[1] > 256:
                mid = jnp.concatenate([mid, lb[r0:r1, 256:]], axis=1)
            parts = ([lb[:r0]] if r0 else []) + [mid] + ([lb[r1:]] if r1 < lb.shape[0] else [])
            return pltpu.bitcast(jnp.concatenate(parts, axis=0) if len(parts) > 1 else mid, BF16)

        def q_rest(n):
            x = pace(x_s[jp, R:], (1, 12, 0, 0)[n])
            w = wq_s[j & 15, :, n * 128:(n + 1) * 128]
            q = (jnp.dot(x, w, preferred_element_type=F32) * SCALE).astype(BF16)
            store_q(j, q, R, n * 128)

        def q_head():
            assert not pending()
            main = jnp.dot(x_s[jp, :R, :DM], wq_s[j & 15, :DM, :], preferred_element_type=F32)
            t = jnp.stack(tails)
            tail = jnp.concatenate(
                [jnp.concatenate([t[:, n * 8:(n + 1) * 8, hf * 128:(hf + 1) * 128] for n in range(4)], axis=2)
                 for hf in range(2)], axis=1).reshape(R, W)
            store_q(j, ((main + tail) * SCALE).astype(BF16), 0, 0)

        def qk(b):
            q = q_s[i & 7, b]
            if pending():
                s = jnp.concatenate(
                    [lax.dot_general(pace(q, 0, 2 if r == 3 else 0), k_s[slot, b, r * 256:(r + 1) * 256, :], NT,
                                     preferred_element_type=F32) for r in range(4)], axis=1)
            else:
                s = lax.dot_general(q, k_s[slot, b], NT, preferred_element_type=F32)
            m = jnp.max(s, axis=-1, keepdims=True)
            pf = jnp.exp2(s - m)
            u = pltpu.bitcast(pf.astype(BF16), U32)
            lp, parts = None, []
            for hf in range(2):
                for c in range(4 * hf, 4 * hf + 4):
                    t = pf[:, c * 128:(c + 1) * 128]
                    lp = t if lp is None else lp + t
                a = halves_on_lanes(pltpu.bitcast(lp, U32)).reshape(SQ, 256)
                parts += [jnp.where(always, u[:, hf * 512:hf * 512 + 256], a),
                          u[:, hf * 512 + 256:hf * 512 + 512]]
            return pltpu.bitcast(jnp.concatenate(parts, axis=1), BF16), lp

        def pv(b, pb, lp):
            if pending():
                o = jnp.concatenate(
                    [jnp.dot(pb, v_s[slot, b, :, :128], preferred_element_type=F32),
                     jnp.dot(jnp.concatenate([pb[:, :512], pace(pb[:, 512:])], axis=1),
                             v_s[slot, b, :, 128:], preferred_element_type=F32)], axis=1)
            else:
                o = jnp.dot(pb, v_s[slot, b], preferred_element_type=F32)
            lp = jnp.where(always, lp, o[:, 0:128])
            if staged:
                zt = staged.pop()
                ls = [lp[:128], lp[128:256], lp[256:]]
                for c in range(4):
                    ls[c % 2] = jnp.where(always, ls[c % 2], zt[:, c * 128:(c + 1) * 128])
                lp = jnp.concatenate(ls, axis=0)
            l = jnp.sum(lp, axis=-1, keepdims=True)
            r = pl.reciprocal(l, approx=True)
            r = r * (2.0 - l * r)
            o = (o * r).astype(BF16)
            o_s[b * SQ:(b + 1) * SQ, :DH] = o[:SQ]
            o_s[b * SQ:(b + 1) * SQ, DH:] = o[SQ:]

        def oproj(n):
            cs = slice(n * 128, (n + 1) * 128)
            part = lax.dot_general(pace(wo_s[i & 15]), o_s[cs, :], NT, preferred_element_type=F32)
            if not final:
                if n >= 6:
                    deps.append(part)
                acc_s[ab, :, cs] = jnp.where(h == 0, 0.0, acc_s[ab, :, cs]) + part
            else:
                fin = acc_s[ab, :, cs] + part
                acc_s[ab, :, cs] = fin
                r = fin[:DR]
                ra = jnp.where(ab == 0, r, mid_s[:, cs])
                mid_s[:, cs] = ra
                zt = jnp.concatenate([fin[DR:], ra, r], axis=0).T
                st_s[p, cs, :] = zt.astype(BF16)
                staged.append(zt)

        def write_back(n):
            r = pl.multiple_of((p >> 1) * T + n * 128, 128)
            c = pl.multiple_of(ab * W, W)

            @pl.when(h == HKV - 1)
            def _():
                copy(st_s.at[p, pl.ds(n * 128, 128), pl.ds(0, DM)],
                     out.at[pl.ds(r, 128), pl.ds(c, DM)], out_sem).start()

            @pl.when(jnp.logical_and(h == HKV - 1, ab == 1))
            def _():
                copy(st_s.at[p, pl.ds(n * 128, 128), pl.ds(DM, 128)],
                     out.at[pl.ds(r, 128), pl.ds(DM, 128)], out_sem).start()

        def prefetch_q_operands(jn):
            n = jnp.minimum(jn, NBLK - 1)
            start_from(jn < 16, (n >> 3) & 1, lambda a: (wq_copy(a, n),))
            start_from(jnp.logical_and(jn < NBLK, (n & 7) == 0), (n >> 3) & 1,
                       lambda a: (x_copy(a, n >> 3),))
            start_from(jn + 1 < LOOK + 16, ((jn + 1) >> 3) & 1, lambda a: (wt_copy(a, jn + 1),))

        live = {}
        for tok in (Y_ORDER if final else X_ORDER).split():
            kind, n = tok[0], int(tok[1:])
            if kind == "k":
                live[n] = qk(n)
            elif kind == "v":
                pv(n, *live.pop(n))
            elif kind == "o":
                oproj(n)
            elif kind == "r":
                q_rest(n)
            elif kind == "z":
                q_head()
            elif kind == "t":
                write_back(n)
            elif kind == "w":
                build_wb(j + 1, always, jnp.concatenate(deps, axis=0))
            elif kind == "b":
                g0 = (p & 1) * (NG // 2)
                build_xb(3 * NG + g0, g0, NG // 2)
            else:
                prefetch_q_operands(j + 2)

    def fence():
        pl.semaphore_signal(bar_sem, 1)
        pl.semaphore_wait(bar_sem, 1)

    half = T // 2
    xh = [copy(xa.at[pl.ds(c * half, half)], x_s.at[0, pl.ds(c * half, half)], x_sem.at[c])
          for c in range(2)]
    wh = [copy(wqa.at[:, pl.ds(c * DH, DH)], wq_s.at[0, :, pl.ds(c * DH, DH)], wq_sem.at[7 * c])
          for c in range(2)]
    for c in range(2):
        xh[c].start()
        wh[c].start()
        fence()
    for c in ([xt_copy(0), xt_copy(1), xt_copy(2), wt_copy(0, LOOK), wt_copy(0, LOOK + 1)]
              + [wq_copy(0, j) for j in range(1, LOOK)]):
        c.start()
    fence()
    for c in kv_copies(0, 0) + wo_copies(0, 0) + (wq_copy(0, LOOK),):
        c.start()
    fence()
    for c in (wq_copy(0, LOOK + 1), wt_copy(0, LOOK + 2), xt_copy(3)):
        c.start()

    def qproj0(rh, ch):
        x = x_s[0, rh * half:(rh + 1) * half]
        w = wq_s[0, :, ch * DH:(ch + 1) * DH]
        q = (jnp.dot(x, w, preferred_element_type=F32) * SCALE).astype(BF16)
        store_q(0, q, rh * half, ch * DH)

    xh[0].wait()
    wh[0].wait()
    qproj0(0, 0)
    xh[1].wait()
    wh[1].wait()
    qproj0(0, 1)
    qproj0(1, 0)
    qproj0(1, 1)
    for c in range(3):
        xt_copy(c).wait()
    wt_copy(0, LOOK).wait()

    ngp = -(-3 * NG // (LOOK - 1))

    def qproj_ahead(jj, carry):
        j = 1 + jj
        wq_copy(0, j).wait()
        g0 = jnp.minimum(jj * ngp, 3 * NG - ngp)
        build_xb(g0, g0, ngp)
        qs = []
        for n in range(4):
            qf = jnp.dot(x_s[0], wq_s[j, :, n * 128:(n + 1) * 128], preferred_element_type=F32)
            qs.append(qf)
            store_q(j, (qf * SCALE).astype(BF16), 0, n * 128)
        build_wb(LOOK, jj >= 0, jnp.concatenate(qs[:2], axis=0))
        return carry
    lax.fori_loop(0, LOOK - 1, qproj_ahead, 0)

    def phase(p, carry):
        nx = jnp.where(p == 3, HKV - (LOOK - 3), HKV - 1)

        def x_body(h, c):
            block(p * HKV + h, False)
            return c
        lax.fori_loop(0, nx, x_body, 0)

        def y_body(h, c):
            block(p * HKV + h, True)
            return c
        lax.fori_loop(nx, HKV, y_body, 0)
        return carry
    lax.fori_loop(0, 4, phase, 0)

    wait_for(out, out_sem)


@jax.jit
def pallas_concat_heads__gqa_block_cached__gqa_block_cached__near_ridge_kernel(
    A_x: jax.Array,
    A_k_cache: jax.Array,
    A_v_cache: jax.Array,
    A_wq: jax.Array,
    A_wo: jax.Array,
    B_x: jax.Array,
    B_k_cache: jax.Array,
    B_v_cache: jax.Array,
    B_wq: jax.Array,
    B_wo: jax.Array,
):
    assert A_x.shape == (B, SQ, D) and A_k_cache.shape == (B, HKV, SK, DH)
    any_spec = pl.BlockSpec(memory_space=pl.ANY)
    out = pl.pallas_call(
        _kernel,
        in_specs=[any_spec] * 10,
        out_specs=any_spec,
        out_shape=jax.ShapeDtypeStruct((B * SQ, 2 * D), BF16),
        scratch_shapes=[
            pltpu.VMEM((4, T, D), BF16),
            pltpu.VMEM((16, D, W), BF16),
            pltpu.VMEM((16, D, W), BF16),
            pltpu.VMEM((2, NB, SK, DH), BF16),
            pltpu.VMEM((2, NB, SK, DH), BF16),
            pltpu.VMEM((8, NB, 2 * SQ, DH), BF16),
            pltpu.VMEM((T, W), BF16),
            pltpu.VMEM((2, D, T), F32),
            pltpu.VMEM((DR, T), F32),
            pltpu.VMEM((4, T, W), BF16),
            pltpu.VMEM((4 * R, DR), BF16),
            pltpu.VMEM((3 * NG, DR, 8, 256), F32),
            pltpu.VMEM((NC, 4, KC, 8, 128), F32),
            pltpu.VMEM((16, DR, W), BF16),
            pltpu.SemaphoreType.DMA((2, 2)),
            pltpu.SemaphoreType.DMA((8,)),
            pltpu.SemaphoreType.DMA((2,)),
            pltpu.SemaphoreType.DMA((4,)),
            pltpu.SemaphoreType.DMA(()),
            pltpu.SemaphoreType.DMA((4,)),
            pltpu.SemaphoreType.DMA((4,)),
            pltpu.SemaphoreType.REGULAR,
        ],
        compiler_params=pltpu.CompilerParams(
            disable_bounds_checks=True,
            vmem_limit_bytes=120 * 1024 * 1024),
    )(A_x.reshape(B * SQ, D), A_k_cache, A_v_cache, A_wq, A_wo.T,
      B_x.reshape(B * SQ, D), B_k_cache, B_v_cache, B_wq, B_wo.T)
    return out.reshape(B, SQ, 2 * D)
```

```python
import jax
import jax.numpy as jnp
from jax import lax
import jax.experimental.pallas as pl
import jax.experimental.pallas.tpu as pltpu

LOG2E = 1.4426950408889634
NT = (((1,), (1,)), ((), ()))

B, SQ, D = 16, 144, 448
HKV, SK, DH = 8, 1024, 256
NB = 8
T = NB * SQ
W = 2 * DH
DM = 384
DR = D - DM
LOOK = 5
NBLK = 32
NG = 32
R = NG * 16
KC = 8
NC = DR // KC

X_ORDER = ("r0 k0 k1 v0 k2 v1 o0 k3 v2 o1 k4 v3 o2 k5 v4 o3 k6 v5 o4 k7 r1 v6 o5 "
           "r2 v7 z0 o6 o7 o8 w0 r3 n0")
Y_ORDER = ("k0 k1 v0 k2 v1 o0 t0 k3 v2 o1 t1 k4 v3 o2 t2 k5 v4 o3 t3 k6 v5 o4 "
           "t4 k7 v6 o5 t5 v7 o6 t6 o7 t7 o8 t8 b0")

F32 = jnp.float32
BF16 = jnp.bfloat16
U32 = jnp.uint32
SCALE = (DH ** -0.5) * LOG2E


def _kernel(xa, ka, va, wqa, wota, xb, kb, vb, wqb, wotb, out,
            x_s, wq_s, wo_s, k_s, v_s, q_s, o_s, acc_s, mid_s, st_s, xt_s, xb_s, wb_s, wt_s,
            kv_sem, wq_sem, wo_sem, x_sem, out_sem, xt_sem, wt_sem, bar_sem):
    srcs = ((xa, ka, va, wqa, wota), (xb, kb, vb, wqb, wotb))
    copy = pltpu.make_async_copy

    def wait_for(dst, sem):
        copy(dst, dst, sem).wait()

    def kv_copies(ab, i):
        g, h, slot = i >> 4, i & 7, i & 1
        return (copy(srcs[ab][1].at[pl.ds(g * NB, NB), h], k_s.at[slot], kv_sem.at[0, slot]),
                copy(srcs[ab][2].at[pl.ds(g * NB, NB), h], v_s.at[slot], kv_sem.at[1, slot]))

    def wq_copy(ab, j):
        c = pl.multiple_of((j & 7) * W, W)
        return copy(srcs[ab][3].at[:, pl.ds(c, W)], wq_s.at[j & 15], wq_sem.at[j & 7])

    def wt_copy(ab, j):
        c = pl.multiple_of((j & 7) * W, W)
        return copy(srcs[ab][3].at[pl.ds(DM, DR), pl.ds(c, W)], wt_s.at[j & 15], wt_sem.at[j & 3])

    def wo_copies(ab, i):
        c = pl.multiple_of((i & 7) * W, W)
        wot, dst, sem = srcs[ab][4], wo_s.at[i & 15], wo_sem.at[i & 1]
        if ab == 1:
            return (copy(wot.at[:, pl.ds(c, W)], dst, sem),)
        return (copy(wot.at[pl.ds(DM, DR), pl.ds(c, W)], dst.at[pl.ds(0, DR)], sem),
                copy(wot.at[pl.ds(0, DM), pl.ds(c, W)], dst.at[pl.ds(DR, DM)], sem))

    def x_copy(ab, p):
        r = pl.multiple_of((p >> 1) * T, T)
        return copy(srcs[ab][0].at[pl.ds(r, T)], x_s.at[p], x_sem.at[p])

    def xt_copy(p):
        return copy(srcs[p & 1][0].at[pl.ds((p >> 1) * T, R), pl.ds(DM, DR)],
                    xt_s.at[pl.ds(p * R, R)], xt_sem.at[p])

    def start_from(cond, ab_dyn, fn):
        for ab in range(2):
            @pl.when(jnp.logical_and(cond, ab_dyn == ab))
            def _():
                for c in fn(ab):
                    c.start()

    def store_q(j, q, row0, col0):
        nrow, ncol = q.shape
        cw = min(ncol, DH)
        for c0 in range(col0, col0 + ncol, cw):
            head, cc = c0 // DH, c0 % DH
            r = row0
            while r < row0 + nrow:
                b, off = r // SQ, r % SQ
                n = min(SQ - off, row0 + nrow - r)
                q_s[j & 7, b, head * SQ + off:head * SQ + off + n, cc:cc + cw] = (
                    q[r - row0:r - row0 + n, c0 - col0:c0 - col0 + cw])
                r += n

    def halves_on_lanes(v):
        v = v.reshape(v.shape[0] // 16, 16, 128)
        return jnp.concatenate([v[:, :8], v[:, 8:]], axis=2)

    def build_xb(gs, gd, ng):
        xt = pltpu.bitcast(xt_s[pl.ds(pl.multiple_of(gs * 16, 16), ng * 16), :], U32)
        for k in range(DR):
            bc = jnp.broadcast_to(xt[:, k:k + 1], (ng * 8, 128))
            xb_s[pl.ds(gd, ng), k] = halves_on_lanes(pltpu.bitcast(bc, BF16).astype(F32))

    def build_wb(j, always, dep):
        w32 = wt_s[j & 15].astype(F32)
        step = dep.shape[0] // 256 * 8
        for c in range(4):
            dc = jnp.concatenate([dep[(c * 8 + r) * step:(c * 8 + r) * step + 8] for r in range(8)], axis=0)
            wc = jnp.where(always, w32[:, c * 128:(c + 1) * 128], dc)
            wb_s[:, c] = jnp.broadcast_to(wc[:, None, :], (DR, 8, 128)).reshape(NC, KC, 8, 128)

    def block(i, final):
        slot, p, h = i & 1, i >> 3, i & 7
        ab = p & 1
        j = i + LOOK - p
        jp = j >> 3

        wait_for(k_s.at[slot], kv_sem.at[0, slot])
        wait_for(v_s.at[slot], kv_sem.at[1, slot])

        @pl.when(i < 16)
        def _():
            wait_for(wo_s.at[i & 15], wo_sem.at[i & 1])
        if not final:
            @pl.when(j < 16)
            def _():
                wait_for(wq_s.at[j & 15], wq_sem.at[j & 7])

            @pl.when((j & 7) == 0)
            def _():
                wait_for(x_s.at[jp], x_sem.at[jp])

            @pl.when(j + 1 < LOOK + 16)
            def _():
                wait_for(wt_s.at[(j + 1) & 15], wt_sem.at[(j + 1) & 3])
        else:
            @pl.when(p == 0)
            def _():
                xt_copy(3).wait()

        nxt = jnp.minimum(i + 1, NBLK - 1)
        start_from(i < NBLK - 1, (nxt >> 3) & 1, lambda a: kv_copies(a, nxt))
        start_from(i < 15, (nxt >> 3) & 1, lambda a: wo_copies(a, nxt))

        always = i >= 0
        staged = []

        groups = [] if final else list(range(NG))
        tails, queue, deps = [], [], []

        def tail_group():
            g = groups.pop(0)
            x = xb_s[jnp.where(jp == 3, 0, jp) * NG + g].reshape(NC, 1, KC, 8, 256)
            w = wb_s[...]
            pr = jnp.sum(x * jnp.concatenate([w, w], axis=4), axis=2).reshape(NC, 32, 256)
            cum = [pr[0]]
            for c in range(1, NC):
                cum.append(cum[-1] + pr[c])
            tails.append(cum[-1])
            queue.append(pltpu.bitcast(jnp.concatenate(cum, axis=0), U32))

        def pending():
            return bool(groups or queue)

        def pace(lhs, skip=0, cut=0):
            if not pending():
                return lhs
            lb = pltpu.bitcast(lhs, U32)
            r0 = r1 = skip * 8
            lim = lb.shape[0] - cut * 8
            got = []
            while r1 < lim and pending():
                if not queue:
                    tail_group()
                a = queue.pop(0)
                n = min(a.shape[0], lim - r1)
                if n < a.shape[0]:
                    queue.append(a[n:])
                    a = a[:n]
                got.append(a)
                r1 += n
            mid = jnp.where(always, lb[r0:r1, :256], jnp.concatenate(got, axis=0) if len(got) > 1 else got[0])
            if lb.shape[1] > 256:
                mid = jnp.concatenate([mid, lb[r0:r1, 256:]], axis=1)
            parts = ([lb[:r0]] if r0 else []) + [mid] + ([lb[r1:]] if r1 < lb.shape[0] else [])
            return pltpu.bitcast(jnp.concatenate(parts, axis=0) if len(parts) > 1 else mid, BF16)

        def q_rest(n):
            x = pace(x_s[jp, R:], (1, 12, 0, 0)[n])
            w = wq_s[j & 15, :, n * 128:(n + 1) * 128]
            q = (jnp.dot(x, w, preferred_element_type=F32) * SCALE).astype(BF16)
            store_q(j, q, R, n * 128)

        def q_head():
            assert not pending()
            main = jnp.dot(x_s[jp, :R, :DM], wq_s[j & 15, :DM, :], preferred_element_type=F32)
            t = jnp.stack(tails)
            tail = jnp.concatenate(
                [jnp.concatenate([t[:, n * 8:(n + 1) * 8, hf * 128:(hf + 1) * 128] for n in range(4)], axis=2)
                 for hf in range(2)], axis=1).reshape(R, W)
            store_q(j, ((main + tail) * SCALE).astype(BF16), 0, 0)

        def qk(b):
            q = q_s[i & 7, b]
            if pending():
                s = jnp.concatenate(
                    [lax.dot_general(pace(q, 0, 2 if r == 3 else 0), k_s[slot, b, r * 256:(r + 1) * 256, :], NT,
                                     preferred_element_type=F32) for r in range(4)], axis=1)
            else:
                s = lax.dot_general(q, k_s[slot, b], NT, preferred_element_type=F32)
            m = jnp.max(s, axis=-1, keepdims=True)
            pf = jnp.exp2(s - m)
            u = pltpu.bitcast(pf.astype(BF16), U32)
            lp, parts = None, []
            for hf in range(2):
                for c in range(4 * hf, 4 * hf + 4):
                    t = pf[:, c * 128:(c + 1) * 128]
                    lp = t if lp is None else lp + t
                a = halves_on_lanes(pltpu.bitcast(lp, U32)).reshape(SQ, 256)
                parts += [jnp.where(always, u[:, hf * 512:hf * 512 + 256], a),
                          u[:, hf * 512 + 256:hf * 512 + 512]]
            return pltpu.bitcast(jnp.concatenate(parts, axis=1), BF16), lp

        def pv(b, pb, lp):
            if pending():
                pb2 = jnp.concatenate([pb[:, :256], pace(pb[:, 256:512]) if b < 3 else pb[:, 256:512],
                                       pace(pb[:, 512:])], axis=1)
                o = jnp.concatenate(
                    [jnp.dot(pb, v_s[slot, b, :, :128], preferred_element_type=F32),
                     jnp.dot(pb2, v_s[slot, b, :, 128:], preferred_element_type=F32)], axis=1)
            else:
                o = jnp.dot(pb, v_s[slot, b], preferred_element_type=F32)
            lp = jnp.where(always, lp, o[:, 0:128])
            if staged:
                zt = staged.pop()
                ls = [lp[:128], lp[128:256], lp[256:]]
                for c in range(4):
                    ls[c % 2] = jnp.where(always, ls[c % 2], zt[:, c * 128:(c + 1) * 128])
                lp = jnp.concatenate(ls, axis=0)
            l = jnp.sum(lp, axis=-1, keepdims=True)
            r = pl.reciprocal(l, approx=True)
            r = r * (2.0 - l * r)
            o = (o * r).astype(BF16)
            o_s[b * SQ:(b + 1) * SQ, :DH] = o[:SQ]
            o_s[b * SQ:(b + 1) * SQ, DH:] = o[SQ:]

        def oproj(n):
            cs = slice(n * 128, (n + 1) * 128)
            part = lax.dot_general(pace(wo_s[i & 15]), o_s[cs, :], NT, preferred_element_type=F32)
            if not final:
                if n >= 6:
                    deps.append(part)
                acc_s[ab, :, cs] = jnp.where(h == 0, 0.0, acc_s[ab, :, cs]) + part
            else:
                fin = acc_s[ab, :, cs] + part
                acc_s[ab, :, cs] = fin
                r = fin[:DR]
                ra = jnp.where(ab == 0, r, mid_s[:, cs])
                mid_s[:, cs] = ra
                zt = jnp.concatenate([fin[DR:], ra, r], axis=0).T
                st_s[p, cs, :] = zt.astype(BF16)
                staged.append(zt)

        def write_back(n):
            r = pl.multiple_of((p >> 1) * T + n * 128, 128)
            c = pl.multiple_of(ab * W, W)

            @pl.when(h == HKV - 1)
            def _():
                copy(st_s.at[p, pl.ds(n * 128, 128), pl.ds(0, DM)],
                     out.at[pl.ds(r, 128), pl.ds(c, DM)], out_sem).start()

            @pl.when(jnp.logical_and(h == HKV - 1, ab == 1))
            def _():
                copy(st_s.at[p, pl.ds(n * 128, 128), pl.ds(DM, 128)],
                     out.at[pl.ds(r, 128), pl.ds(DM, 128)], out_sem).start()

        def prefetch_q_operands(jn):
            n = jnp.minimum(jn, NBLK - 1)
            start_from(jn < 16, (n >> 3) & 1, lambda a: (wq_copy(a, n),))
            start_from(jnp.logical_and(jn < NBLK, (n & 7) == 0), (n >> 3) & 1,
                       lambda a: (x_copy(a, n >> 3),))
            start_from(jn + 1 < LOOK + 16, ((jn + 1) >> 3) & 1, lambda a: (wt_copy(a, jn + 1),))

        live = {}
        for tok in (Y_ORDER if final else X_ORDER).split():
            kind, n = tok[0], int(tok[1:])
            if kind == "k":
                live[n] = qk(n)
            elif kind == "v":
                pv(n, *live.pop(n))
            elif kind == "o":
                oproj(n)
            elif kind == "r":
                q_rest(n)
            elif kind == "z":
                q_head()
            elif kind == "t":
                write_back(n)
            elif kind == "w":
                build_wb(j + 1, always, jnp.concatenate(deps, axis=0))
            elif kind == "b":
                g0 = (p & 1) * (NG // 2)
                build_xb(3 * NG + g0, g0, NG // 2)
            else:
                prefetch_q_operands(j + 2)

    def fence():
        pl.semaphore_signal(bar_sem, 1)
        pl.semaphore_wait(bar_sem, 1)

    half = T // 2
    xh = [copy(xa.at[pl.ds(c * half, half)], x_s.at[0, pl.ds(c * half, half)], x_sem.at[c])
          for c in range(2)]
    wh = [copy(wqa.at[:, pl.ds(c * DH, DH)], wq_s.at[0, :, pl.ds(c * DH, DH)], wq_sem.at[7 * c])
          for c in range(2)]
    for c in range(2):
        xh[c].start()
        wh[c].start()
        fence()
    for c in ([xt_copy(0), xt_copy(1), xt_copy(2), wt_copy(0, LOOK), wt_copy(0, LOOK + 1)]
              + [wq_copy(0, j) for j in range(1, LOOK)]):
        c.start()
    fence()
    for c in kv_copies(0, 0) + wo_copies(0, 0) + (wq_copy(0, LOOK),):
        c.start()
    fence()
    for c in (wq_copy(0, LOOK + 1), wt_copy(0, LOOK + 2), xt_copy(3)):
        c.start()

    def qproj0(rh, ch):
        x = x_s[0, rh * half:(rh + 1) * half]
        w = wq_s[0, :, ch * DH:(ch + 1) * DH]
        q = (jnp.dot(x, w, preferred_element_type=F32) * SCALE).astype(BF16)
        store_q(0, q, rh * half, ch * DH)

    xh[0].wait()
    wh[0].wait()
    qproj0(0, 0)
    xh[1].wait()
    wh[1].wait()
    qproj0(0, 1)
    qproj0(1, 0)
    qproj0(1, 1)
    for c in range(3):
        xt_copy(c).wait()
    wt_copy(0, LOOK).wait()

    ngp = -(-3 * NG // (LOOK - 1))

    def qproj_ahead(jj, carry):
        j = 1 + jj
        wq_copy(0, j).wait()
        g0 = jnp.minimum(jj * ngp, 3 * NG - ngp)
        build_xb(g0, g0, ngp)
        qs = []
        for n in range(4):
            qf = jnp.dot(x_s[0], wq_s[j, :, n * 128:(n + 1) * 128], preferred_element_type=F32)
            qs.append(qf)
            store_q(j, (qf * SCALE).astype(BF16), 0, n * 128)
        build_wb(LOOK, jj >= 0, jnp.concatenate(qs[:2], axis=0))
        return carry
    lax.fori_loop(0, LOOK - 1, qproj_ahead, 0)

    def phase(p, carry):
        nx = jnp.where(p == 3, HKV - (LOOK - 3), HKV - 1)

        def x_body(h, c):
            block(p * HKV + h, False)
            return c
        lax.fori_loop(0, nx, x_body, 0)

        def y_body(h, c):
            block(p * HKV + h, True)
            return c
        lax.fori_loop(nx, HKV, y_body, 0)
        return carry
    lax.fori_loop(0, 4, phase, 0)

    wait_for(out, out_sem)


@jax.jit
def pallas_concat_heads__gqa_block_cached__gqa_block_cached__near_ridge_kernel(
    A_x: jax.Array,
    A_k_cache: jax.Array,
    A_v_cache: jax.Array,
    A_wq: jax.Array,
    A_wo: jax.Array,
    B_x: jax.Array,
    B_k_cache: jax.Array,
    B_v_cache: jax.Array,
    B_wq: jax.Array,
    B_wo: jax.Array,
):
    assert A_x.shape == (B, SQ, D) and A_k_cache.shape == (B, HKV, SK, DH)
    any_spec = pl.BlockSpec(memory_space=pl.ANY)
    out = pl.pallas_call(
        _kernel,
        in_specs=[any_spec] * 10,
        out_specs=any_spec,
        out_shape=jax.ShapeDtypeStruct((B * SQ, 2 * D), BF16),
        scratch_shapes=[
            pltpu.VMEM((4, T, D), BF16),
            pltpu.VMEM((16, D, W), BF16),
            pltpu.VMEM((16, D, W), BF16),
            pltpu.VMEM((2, NB, SK, DH), BF16),
            pltpu.VMEM((2, NB, SK, DH), BF16),
            pltpu.VMEM((8, NB, 2 * SQ, DH), BF16),
            pltpu.VMEM((T, W), BF16),
            pltpu.VMEM((2, D, T), F32),
            pltpu.VMEM((DR, T), F32),
            pltpu.VMEM((4, T, W), BF16),
            pltpu.VMEM((4 * R, DR), BF16),
            pltpu.VMEM((3 * NG, DR, 8, 256), F32),
            pltpu.VMEM((NC, 4, KC, 8, 128), F32),
            pltpu.VMEM((16, DR, W), BF16),
            pltpu.SemaphoreType.DMA((2, 2)),
            pltpu.SemaphoreType.DMA((8,)),
            pltpu.SemaphoreType.DMA((2,)),
            pltpu.SemaphoreType.DMA((4,)),
            pltpu.SemaphoreType.DMA(()),
            pltpu.SemaphoreType.DMA((4,)),
            pltpu.SemaphoreType.DMA((4,)),
            pltpu.SemaphoreType.REGULAR,
        ],
        compiler_params=pltpu.CompilerParams(
            disable_bounds_checks=True,
            vmem_limit_bytes=120 * 1024 * 1024),
    )(A_x.reshape(B * SQ, D), A_k_cache, A_v_cache, A_wq, A_wo.T,
      B_x.reshape(B * SQ, D), B_k_cache, B_v_cache, B_wq, B_wo.T)
    return out.reshape(B, SQ, 2 * D)
```
